```python
import os as _os
_os.environ.setdefault('JAX_PLATFORMS', 'cpu')
import jax
import jax.numpy as jnp

def _softmax(x, axis=-1):
    return jax.nn.softmax(x, axis=axis)

def _gelu(x):
    return jax.nn.gelu(x, approximate=True)

def _silu(x):
    return jax.nn.silu(x)

def _sigmoid(x):
    return jax.nn.sigmoid(x)

def _layernorm(x, axis=-1, eps=1e-05):
    m = jnp.mean(x, axis=axis, keepdims=True)
    v = jnp.var(x, axis=axis, keepdims=True)
    return (x - m) / jnp.sqrt(v + eps)

def _scatter_add(tgt, idx, src, axis=0):
    return tgt.at[idx].add(src)

def _segment_sum(src, seg, n):
    return jax.ops.segment_sum(src, seg, n)

class _Rng:

    def __init__(self, key):
        self._k = key

    def _next(self):
        self._k, sub = jax.random.split(self._k)
        return sub

    def normal(self, shape):
        return jax.random.normal(self._next(), shape, dtype=jnp.bfloat16)

    def randint(self, lo, hi, shape):
        return jax.random.randint(self._next(), shape, lo, hi, dtype=jnp.int32)

    def uniform(self, shape, lo=0.0, hi=1.0):
        return jax.random.uniform(self._next(), shape, jnp.bfloat16, lo, hi)

    def permutation(self, n):
        return jax.random.permutation(self._next(), n)
kernel_name = 'recurrent_scan__memory_aug_recurrent_mem_tr__mixer_gmlp__prompt'

def setup_inputs():
    _rng = _Rng(jax.random.key(int.from_bytes(__import__("os").urandom(4), "little")))
    _w = lambda a: (lambda t: t.astype(jnp.bfloat16) if jnp.issubdtype(t.dtype, jnp.floating) else t)(jnp.asarray(a))

    def _A_setup():
        B, S, Dm = (1, 2048, 640)
        H, Dh = (32, 128)
        M, seg = (8, 32)
        seg = min(seg, S)
        S = S // seg * seg
        return {'x': _w((lambda *s: _rng.normal(s) * 0.05)(B, S, Dm)), 'mem0': _w((lambda *s: _rng.normal(s) * 0.1)(B, M, Dm)), 'Wq': _w((lambda *s: _rng.normal(s) * 1.6)(Dm, H, Dh) * Dm ** (-0.5)), 'Wk': _w((lambda *s: _rng.normal(s) * 1.6)(Dm, H, Dh) * Dm ** (-0.5)), 'Wv': _w((lambda *s: _rng.normal(s) * 0.1)(Dm, H, Dh) * Dm ** (-0.5)), 'Wo': _w((lambda *s: _rng.normal(s) * 0.1)(H, Dh, Dm) * (H * Dh) ** (-0.5)), 'seg_len': seg}
    _A_in = _A_setup()

    def _B_setup():
        B, S, D, F = (1, 2048, 640, 1728)
        Fh = F // 2
        return {'x': _w((lambda *s: _rng.normal(s) * 0.05)(B, S, D)), 'w_in': _w((lambda *s: _rng.normal(s) * 0.8)(D, 2 * Fh)), 'w_sp': _w(0.01 * (lambda *s: _rng.normal(s) * 0.8)(S, S)), 'b_sp': _w(1.0 + 0.01 * (lambda *s: _rng.normal(s) * 0.05)(S)), 'w_out': _w((lambda *s: _rng.normal(s) * 0.05)(Fh, D))}
    _B_in = _B_setup()
    return {'A_x': _A_in['x'], 'A_mem0': _A_in['mem0'], 'A_Wq': _A_in['Wq'], 'A_Wk': _A_in['Wk'], 'A_Wv': _A_in['Wv'], 'A_Wo': _A_in['Wo'], 'A_seg_len': _A_in['seg_len'], 'B_x': _B_in['x'], 'B_w_in': _B_in['w_in'], 'B_w_sp': _B_in['w_sp'], 'B_b_sp': _B_in['b_sp'], 'B_w_out': _B_in['w_out']}

def reference(A_x, A_mem0, A_Wq, A_Wk, A_Wv, A_Wo, A_seg_len, B_x, B_w_in, B_w_sp, B_b_sp, B_w_out):

    def _A_ref(x, mem0, Wq, Wk, Wv, Wo, seg_len):
        B, S, Dm = x.shape
        H, Dh = (Wq.shape[1], Wq.shape[2])
        M = mem0.shape[1]
        scale = Dh ** (-0.5)
        n_seg = S // seg_len
        L = M + seg_len
        idx = jnp.arange(L)
        mask = (idx[:, None] < M) | (idx[:, None] >= idx[None, :])
        mem = mem0
        outs = []
        for s in range(n_seg):
            xs = x[:, s * seg_len:(s + 1) * seg_len, :].copy()
            h = jnp.concatenate([mem, xs], axis=1)
            q = jnp.einsum('btd,dhe->bhte', h, Wq)
            k = jnp.einsum('btd,dhe->bhte', h, Wk)
            v = jnp.einsum('btd,dhe->bhte', h, Wv)
            scores = jnp.einsum('bhqe,bhke->bhqk', q, k) * scale
            scores = jnp.where(mask[None, None], scores, -1000000000.0)
            p = _softmax(scores, axis=-1)
            o = jnp.einsum('bhqk,bhke->bhqe', p, v)
            o = jnp.einsum('bhte,hed->btd', o, Wo)
            mem = o[:, :M, :].copy()
            outs.append(o[:, M:, :])
        return jnp.concatenate(outs, axis=1)

    def _B_ref(x, w_in, w_sp, b_sp, w_out):
        B, S, D = x.shape
        F = w_in.shape[-1]
        Fh = F // 2
        z = _gelu(jnp.einsum('bsd,df->bsf', x, w_in))
        z1 = z[..., :Fh].copy()
        z2 = _layernorm(z[..., Fh:], axis=-1)
        g = jnp.einsum('ts,bsf->btf', w_sp, z2) + b_sp[None, :, None]
        return jnp.einsum('bsf,fd->bsd', z1 * g, w_out)
    x = A_x
    xn = _layernorm(x, axis=-1)
    s = _A_ref(xn, A_mem0, A_Wq, A_Wk, A_Wv, A_Wo, A_seg_len)
    g = _silu(_B_ref(xn, B_w_in, B_w_sp, B_b_sp, B_w_out))
    return x + s * g
```

```python
import functools
import math

import jax
import jax.numpy as jnp
from jax import lax
import jax.experimental.pallas as pl
import jax.experimental.pallas.tpu as pltpu

F32 = jnp.float32
BF16 = jnp.bfloat16
U32 = jnp.uint32
LANES = 128
LOG2E = 1.4426950408889634
EPS = 1e-5
NT = (((1,), (1,)), ((), ()))

CFG = dict(
    tb1=128,
    unroll1=1,
    unroll2=1,
    unrolla=1,
    rc1=96,
    rc2=96,
    order="K0,S1,Q0,P2,V0,O18",
    och=2,
)


def _gelu(x):
    c0 = math.sqrt(2.0 / math.pi)
    u = x * (c0 + (c0 * 0.044715) * (x * x))
    return (0.5 * x) * (1.0 + jnp.tanh(u))


def _as_bf16(words):
    return pltpu.bitcast(words, BF16)


def _as_words(x):
    return pltpu.bitcast(x.astype(BF16), U32)


def _dot(a, b):
    return jnp.dot(a, b, preferred_element_type=F32)


def _dot_nt(a, b):
    return lax.dot_general(a, b, NT, preferred_element_type=F32)


def _loop(n, unroll, body, init=None):
    if unroll >= n:
        c = init
        for i in range(n):
            c = body(i, c)
        return c
    assert n % unroll == 0

    def outer(o, c):
        for u in range(unroll):
            c = body(o * unroll + u, c)
        return c

    return lax.fori_loop(0, n // unroll, outer, init)


def _rows(i, n):
    if isinstance(i, int):
        return pl.ds(i * n, n)
    return pl.ds(pl.multiple_of(i * n, n), n)


def _kernel(
    x_hbm, mem_hbm, wq_hbm, wk_hbm, wv_hbm, wo_hbm, wint_hbm, wsp_hbm, b_hbm, wout_hbm,
    out_hbm,
    x_v, xn32, xn16, mem_v, wint_v, wsp_v, wout_v, woutt, b_v, b32,
    z2raw, z2t, yt, gate, wqkv, wo_v, wo32, o_scr, out_v,
    sem_x, sem_w, sem_sp, sem_a, sem_o,
    *, seg, cfg,
):
    S, D = x_v.shape
    M = mem_v.shape[0]
    H = wqkv.shape[1]
    DH = wqkv.shape[3]
    FH = wout_v.shape[0]
    NTB = S // LANES
    NP = H // 2
    L = M + seg
    nseg = S // seg
    assert NP == NTB

    def x_copy(i):
        return pltpu.make_async_copy(x_hbm.at[_rows(i, LANES)], x_v.at[_rows(i, LANES)], sem_x.at[i])

    def wsp_copy(i):
        return pltpu.make_async_copy(wsp_hbm.at[_rows(i, LANES)], wsp_v.at[_rows(i, LANES)], sem_sp.at[i])

    def attn_copies(j):
        cps = []
        for i, w in enumerate((wq_hbm, wk_hbm, wv_hbm)):
            w32 = w.bitcast(U32)
            for b in range(2):
                cps.append(pltpu.make_async_copy(w32.at[:, b, j, :], wqkv.at[i, 2 * j + b], sem_a.at[j]))
        cps.append(pltpu.make_async_copy(wo_hbm.at[_rows(j, 2 * DH)], wo_v.at[_rows(j, 2 * DH)], sem_a.at[j]))
        return cps

    w2_copy = pltpu.make_async_copy(wint_hbm.at[pl.ds(FH, FH)], wint_v.at[pl.ds(FH, FH)], sem_w.at[0])
    w1_copy = pltpu.make_async_copy(wint_hbm.at[pl.ds(0, FH)], wint_v.at[pl.ds(0, FH)], sem_w.at[1])
    wout_copy = pltpu.make_async_copy(wout_hbm, wout_v, sem_w.at[2])
    b_copy = pltpu.make_async_copy(b_hbm, b_v, sem_w.at[3])
    mem_copy = pltpu.make_async_copy(mem_hbm, mem_v, sem_w.at[4])

    x_copy(0).start()
    w2_copy.start()
    for i in range(1, NTB):
        x_copy(i).start()
    for c in (w1_copy, wout_copy, b_copy, mem_copy):
        c.start()

    def norm_x(i):
        x = x_v[_rows(i, LANES), :].astype(F32)
        m = jnp.mean(x, axis=-1, keepdims=True)
        d = x - m
        v = jnp.mean(d * d, axis=-1, keepdims=True)
        xn = d * lax.rsqrt(v + EPS)
        xn32[_rows(i, LANES), :] = xn
        xn16[_rows(i, LANES // 2), :] = _as_words(xn)

    def z2_matmul(i):
        rc = cfg["rc1"]
        rhs = _as_bf16(xn16[_rows(i, LANES // 2), :])
        for c in range(FH // rc):
            z = _dot_nt(wint_v[pl.ds(FH + c * rc, rc), :], rhs)
            z2raw[i % 2, pl.ds(c * rc, rc), :] = _gelu(z)

    def z2_norm(i):
        z = z2raw[i % 2]
        m = jnp.mean(z, axis=0, keepdims=True)
        d = z - m
        v = jnp.mean(d * d, axis=0, keepdims=True)
        z2t[i] = _as_words(d * lax.rsqrt(v + EPS))

    x_copy(0).wait()
    norm_x(0)
    x_copy(1).wait()
    w2_copy.wait()
    wsp_copy(0).start()
    norm_x(1)
    z2_matmul(0)

    def phase1(i, _):
        x_copy(i + 1).wait()
        wsp_copy(i).start()
        norm_x(i + 1)
        z2_matmul(i)
        z2_norm(i - 1)

    _loop(NTB - 2, cfg["unroll1"], lambda i, c: phase1(i + 1, c))
    wsp_copy(NTB - 1).start()
    for j in range(2):
        for c in attn_copies(j):
            c.start()
    for c in (w1_copy, wout_copy, b_copy, mem_copy):
        c.wait()
    z2_matmul(NTB - 1)
    z2_norm(NTB - 2)
    b32[...] = b_v[...].astype(F32)
    woutt[...] = _as_words(wout_v[...].astype(F32).T)
    z2_norm(NTB - 1)

    def mix(i):
        rc = cfg["rc2"]
        xb = _as_bf16(xn16[_rows(i, LANES // 2), :])
        wb = wsp_v[_rows(i, LANES), :]
        bias = b32[pl.ds(i, 1), :]
        for c in range(FH // rc):
            z1 = _dot_nt(wint_v[pl.ds(c * rc, rc), :], xb)
            lhs = jnp.concatenate(
                [_as_bf16(z2t[sb, pl.ds(c * rc // 2, rc // 2), :]) for sb in range(NTB)], axis=1)
            g = _dot_nt(lhs, wb)
            yt[i % 2, pl.ds(c * rc // 2, rc // 2), :] = _as_words(_gelu(z1) * (g + bias))

    def gate_out(i):
        y = _as_bf16(yt[i % 2])
        for dc in range(D // LANES):
            o = _dot(_as_bf16(woutt[pl.ds(dc * LANES // 2, LANES // 2), :]), y)
            gate[_rows(i, LANES), pl.ds(dc * LANES, LANES)] = (o * jax.nn.sigmoid(o)).T

    def repack(j):
        for i in range(3):
            a = wqkv[i, 2 * j]
            b = wqkv[i, 2 * j + 1]
            wqkv[i, 2 * j] = (a & U32(0xFFFF)) | (b << 16)
            wqkv[i, 2 * j + 1] = (a >> 16) | (b & U32(0xFFFF0000))
        wo32[_rows(j, DH), :] = pltpu.bitcast(wo_v[_rows(j, 2 * DH), :], U32)

    def phase2(i, first=False, prefetch=True):
        wsp_copy(i).wait()
        for c in attn_copies(i):
            c.wait()
        if prefetch:
            for c in attn_copies(i + 2):
                c.start()
        if not first:
            gate_out(i - 1)
        mix(i)
        repack(i)

    phase2(0, first=True)
    _loop(NTB - 4, cfg["unroll2"], lambda i, c: phase2(i + 1))
    phase2(NTB - 3)
    phase2(NTB - 2, prefetch=False)
    phase2(NTB - 1, prefetch=False)
    gate_out(NTB - 1)

    G = 2
    R = G * L
    NG = H // G
    row = lax.broadcasted_iota(jnp.int32, (R, R), 0)
    col = lax.broadcasted_iota(jnp.int32, (R, R), 1)
    rb = (row >= L).astype(jnp.int32)
    cb = (col >= L).astype(jnp.int32)
    ri = row - rb * L
    ci = col - cb * L
    same_head = rb == cb
    keep = same_head & ((ri < M) | (ri >= ci))
    fill = jnp.where(same_head, -1e9 * LOG2E, -jnp.inf).astype(F32)
    scale = DH ** -0.5 * LOG2E
    order = [(t[0], int(t[1:])) for t in cfg["order"].split(",")]
    och = cfg["och"]

    def step(s, mem):
        h = jnp.concatenate([mem, xn32[_rows(s, seg), :]], axis=0)
        st = {}
        acc = [None]

        def proj(i, g):
            return jnp.concatenate([_dot(h, _as_bf16(wqkv[i, G * g + j])) for j in range(G)], axis=0)

        def do(op, g):
            if g < 0 or g >= NG:
                return
            if op == "Q":
                st["q", g] = proj(0, g)
            elif op == "K":
                st["k", g] = proj(1, g).astype(BF16)
            elif op == "V":
                st["v", g] = proj(2, g).astype(BF16)
            elif op == "S":
                sc = _dot_nt(st.pop(("q", g)), st.pop(("k", g)))
                sc = jnp.where(keep, sc * scale, fill)
                p = jnp.exp2(sc - jnp.max(sc, axis=1, keepdims=True))
                st["p", g] = p * (1.0 / jnp.sum(p, axis=1, keepdims=True))
            elif op == "P":
                o = _dot(st.pop(("p", g)), st.pop(("v", g)))
                for j in range(G):
                    o_scr[:, pl.ds((G * g + j) * DH, DH)] = o[j * L:(j + 1) * L]
            elif op == "O":
                for hd in range(G * g, G * (g + 1), och):
                    y = _dot(o_scr[:, pl.ds(hd * DH, och * DH)],
                             _as_bf16(wo32[pl.ds(hd * DH // 2, och * DH // 2), :]))
                    acc[0] = y if acc[0] is None else acc[0] + y

        for t in range(NG + max(lag for _, lag in order)):
            for op, lag in order:
                do(op, t - lag)
        out = acc[0]
        rows = _rows(s, seg)
        out_v[rows, :] = (x_v[rows, :].astype(F32) + out[M:] * gate[rows, :]).astype(out_v.dtype)
        pltpu.make_async_copy(out_v.at[rows], out_hbm.at[rows], sem_o.at[0]).start()
        return out[:M]

    _loop(nseg, cfg["unrolla"], step, mem_v[...].astype(F32))
    pltpu.make_async_copy(out_v, out_hbm, sem_o.at[0]).wait()


def build(cfg):
    def fn(A_x, A_mem0, A_Wq, A_Wk, A_Wv, A_Wo, A_seg_len, B_x, B_w_in, B_w_sp, B_b_sp, B_w_out):
        del B_x
        B, S, D = A_x.shape
        M = A_mem0.shape[1]
        H, DH = A_Wq.shape[1], A_Wq.shape[2]
        FH = B_w_out.shape[0]
        seg = int(A_seg_len)
        assert B == 1 and DH == LANES
        ntb = S // LANES
        vmem = pltpu.VMEM
        scratch = [
            vmem((S, D), BF16),
            vmem((S, D), F32),
            vmem((S // 2, D), U32),
            vmem((M, D), BF16),
            vmem((2 * FH, D), BF16),
            vmem((S, S), BF16),
            vmem((FH, D), BF16),
            vmem((D // 2, FH), U32),
            vmem((ntb, LANES), BF16),
            vmem((ntb, LANES), F32),
            vmem((2, FH, LANES), F32),
            vmem((ntb, FH // 2, LANES), U32),
            vmem((2, FH // 2, LANES), U32),
            vmem((S, D), F32),
            vmem((3, H, D // 2, DH), U32),
            vmem((H * DH, D), BF16),
            vmem((H * DH // 2, D), U32),
            vmem((M + seg, H * DH), F32),
            vmem((S, D), A_x.dtype),
            pltpu.SemaphoreType.DMA((ntb,)),
            pltpu.SemaphoreType.DMA((5,)),
            pltpu.SemaphoreType.DMA((ntb,)),
            pltpu.SemaphoreType.DMA((H // 2,)),
            pltpu.SemaphoreType.DMA((1,)),
        ]
        hbm = pl.BlockSpec(memory_space=pltpu.HBM)
        out = pl.pallas_call(
            functools.partial(_kernel, seg=seg, cfg=cfg),
            out_shape=jax.ShapeDtypeStruct((S, D), A_x.dtype),
            in_specs=[hbm] * 10,
            out_specs=hbm,
            scratch_shapes=scratch,
            compiler_params=pltpu.CompilerParams(vmem_limit_bytes=110 * 2**20),
        )(
            A_x.reshape(S, D),
            A_mem0.reshape(M, D),
            A_Wq.reshape(D // 2, 2, H, DH),
            A_Wk.reshape(D // 2, 2, H, DH),
            A_Wv.reshape(D // 2, 2, H, DH),
            A_Wo.reshape(H * DH, D),
            B_w_in.T,
            B_w_sp,
            B_b_sp.reshape(ntb, LANES),
            B_w_out,
        )
        return out.reshape(B, S, D)

    return fn


@functools.partial(jax.jit, static_argnames=("A_seg_len",))
def pallas_recurrent_scan__memory_aug_recurrent_mem_tr__mixer_gmlp__prompt_kernel(
    A_x, A_mem0, A_Wq, A_Wk, A_Wv, A_Wo, A_seg_len, B_x, B_w_in, B_w_sp, B_b_sp, B_w_out,
):
    return build(CFG)(A_x, A_mem0, A_Wq, A_Wk, A_Wv, A_Wo, A_seg_len, B_x, B_w_in, B_w_sp, B_b_sp, B_w_out)
```

```python
import functools
import math

import jax
import jax.numpy as jnp
from jax import lax
import jax.experimental.pallas as pl
import jax.experimental.pallas.tpu as pltpu

F32 = jnp.float32
BF16 = jnp.bfloat16
U32 = jnp.uint32
LANES = 128
LOG2E = 1.4426950408889634
EPS = 1e-5
NT = (((1,), (1,)), ((), ()))

CFG = dict(
    unroll=4,
    lnrows=16,
    ln2a=8,
    ln1a=10,
    lnpin=2,
    rprows=8,
    dc=128,
    rc1=96,
    rc2=96,
    lat_s=230,
    lat_p=550,
    lat_o=190,
    hn=8,
    kfirst=6,
    osplit=2,
    porder="nat",
    pre="inline",
    flags="",
    skip="",
    clusters="4,6,5,4,7",
    pin=1,
    sumcost=70,
    opq=0,
    ldmode="val",
    stmode="val",
)

_SCHEME = """
+Q0 | +00 -20 -30 -04 -01 +10 | +S0
+R0 | +00 -02 -03 -40 +01 -10 | +U0
+Q1 | +11 -21 -31 -14 +32 | +S1
+R1 | +11 -12 -13 -41 +23 | +U1
+R2 | -22 +20 +21 +42 -10 | +V2
+P2 | +22 -02 -12 -24 +01 | +S2
+R3 | -33 +30 +31 +43 -32 +23 | +V3
+P3 | +33 -03 -13 -34 -32 +23 | +S3
+Q4 | +44 -40 -41 -24 -34 | +V4
+P4 | +44 -04 -14 -42 -43 | +U4
+Q0 +Q2 | +20 -10 | +V0 +V2
+P0 +P2 | +02 -01 | +U0 +U2
+Q0 +P2 | -02 +20 +01 -10 | +U0 -V2
+Q0 +Q3 | +30 | +V0 +V3
+P0 +P3 | +03 | +U0 +U3
+Q0 +P3 | -03 +30 | +U0 -V3
+R0 +R4 | -40 | +V0 +V4
+P0 +P4 | +04 | +S0 +S4
+R0 +P4 | -04 +40 | +S0 +V4
+R0 +R1 +R2 | -10 | +V0 +V1 +V2
+P0 +P1 +P2 | +01 | +S0 +S1 +S2
+R0 +P1 +P2 | -01 +10 | +S0 +V1 +V2
+Q1 +Q2 | +21 -10 -32 | +V1 +V2
+P1 +P2 | +12 -01 -23 | +U1 +U2
+Q1 +P2 | -12 +21 | +U1 -V2
+Q3 +Q1 +Q2 | +32 | +S3 +S1 +S2
+R3 +R1 +R2 | +23 | +U3 +U1 +U2
+R3 -Q1 -Q2 | +32 -23 | +S3 +U1 +U2
+Q1 +Q3 | +31 -32 | +V1 +V3
+P1 +P3 | +13 -23 | +U1 +U3
+Q1 +P3 | -13 +31 -32 +23 | +U1 -V3
+R1 +R4 | -41 | +V1 +V4
+P1 +P4 | +14 | +S1 +S4
+R1 +P4 | -14 +41 | +S1 +V4
+Q2 +Q4 | +24 | +S2 +S4
+R2 +R4 | +42 | +U2 +U4
+R2 -Q4 | +24 -42 | +S2 +U4
+Q3 +Q4 | +34 | +S3 +S4
+R3 +R4 | +43 | +U3 +U4
+R3 -Q4 | +34 -43 | +S3 +U4
"""
NB = 5


def _parse_scheme():
    sign = {"+": 1, "-": -1}
    products, slots = [], 0
    for line in _SCHEME.strip().split("\n"):
        left, weight, out = (part.split() for part in line.split("|"))
        left = [(sign[t[0]], t[1], int(t[2])) for t in left]
        weight = [(sign[t[0]], int(t[1]), int(t[2])) for t in weight]
        out = [(sign[t[0]], t[1], int(t[2])) for t in out]
        if len(weight) == 1:
            out = [(s * weight[0][0], b, n) for s, b, n in out]
            products.append((left, weight, out, None))
        else:
            products.append((left, sorted(weight, reverse=True), out, slots))
            slots += 1
    return products, slots


def _signed_sum(terms):
    terms = sorted(terms, key=lambda t: -t[0])
    total = terms[0][1] if terms[0][0] > 0 else -terms[0][1]
    for s, v in terms[1:]:
        total = total + v if s > 0 else total - v
    return total


def _gelu_tanh(x):
    c0 = math.sqrt(2.0 / math.pi)
    return jnp.tanh(x * (c0 + (c0 * 0.044715) * (x * x)))


def _dot(a, b):
    return jnp.dot(a, b, preferred_element_type=F32)


def _dot_nt(a, b):
    return lax.dot_general(a, b, NT, preferred_element_type=F32)


def _rows(i, n):
    if isinstance(i, int):
        return pl.ds(i * n, n)
    return pl.ds(pl.multiple_of(i * n, n), n)


class _Packed:
    def __init__(self, words, ldmode, stmode):
        self.words = words
        self.ldmode, self.stmode = ldmode, stmode

    def _index(self, idx):
        idx = idx if isinstance(idx, tuple) else (idx,)
        rank = len(self.words.shape)
        if idx == (Ellipsis,) or len(idx) <= rank - 2:
            return idx
        rows = idx[rank - 2]
        if isinstance(rows, slice):
            assert rows == slice(None)
            return idx
        start = rows.start // 2
        if not isinstance(start, int):
            start = pl.multiple_of(start, 8)
        return idx[:rank - 2] + (pl.ds(start, rows.size // 2),) + idx[rank - 1:]

    def __getitem__(self, idx):
        if self.ldmode == "ref":
            return self.words.bitcast(BF16)[idx]
        return pltpu.bitcast(self.words[self._index(idx)], BF16)

    def __setitem__(self, idx, value):
        if self.stmode == "ref":
            self.words.bitcast(BF16)[idx] = value
        else:
            self.words[self._index(idx)] = pltpu.bitcast(value, U32)


class _Stream:
    def __init__(self):
        self.now = 0
        self.waiting = []

    def defer(self, ready, cost, fn):
        self.waiting.append((ready, cost, fn))
        self.waiting.sort(key=lambda w: w[0])

    def _emit_next(self):
        ready, cost, fn = self.waiting.pop(0)
        self.now = max(self.now, ready) + cost
        fn()

    def run(self, cost, fn):
        while self.waiting and self.waiting[0][0] <= self.now:
            self._emit_next()
        self.now += cost
        return fn()

    def until(self, done):
        while not done():
            self._emit_next()


def _kernel(
    x_hbm, mem_hbm, wq_hbm, wk_hbm, wv_hbm, wo_hbm, wint_hbm, wsp_hbm, b_hbm, wout_hbm,
    out_hbm,
    x_v, x0_v, xn_w, s0_w, s1_w, s2_w, s3_w, mem_v, wint_v, wsp_v, wout_v, woutt_w, b_v, b32,
    zt, d0_v, d1_v, z2_w, ws0_w, ws1_w, ws2_w, ws3_w, yta_w, ytb_w, gate, wqkv_w, wo_v, wo_w, wfq_w, wfo_w,
    lq_w, lo_w, qkv_carry, o_carry, o16_w, o32, out_v, zero,
    sem_x, sem_w, sem_sp, sem_wo, sem_a, sem_o,
    *, seg, cfg,
):
    S, D = out_v.shape
    M = mem_v.shape[0]
    H = o_carry.shape[0]
    DH = LANES
    FH = wout_v.shape[0]
    NTB = S // LANES
    NN = D // LANES
    L = M + seg
    U = cfg["unroll"]
    NIT = NTB // U
    assert (M, seg, NN, H // 2) == (8, 32, NB, NTB)
    products, _ = _parse_scheme()
    sums = [(weight, slot) for _, weight, _, slot in products if slot is not None]
    sizes = [int(t) for t in cfg["clusters"].split(",")]
    assert sum(sizes) == len(sums)
    clusters = [sums[sum(sizes[:e]):sum(sizes[:e + 1])] for e in range(len(sizes))]
    n_fo = H // NB
    h_rest = H - NB * n_fo

    xn, woutt, yta, ytb, wqkv, wo, wfq, wfo, lq, lo, o16 = (
        _Packed(r, cfg["ldmode"], cfg["stmode"]) for r in (xn_w, woutt_w, yta_w, ytb_w, wqkv_w, wo_w, wfq_w, wfo_w, lq_w, lo_w, o16_w))

    stage_w = (s0_w, s1_w, s2_w, s3_w)
    z2 = _Packed(z2_w, 'val', 'val')
    ws_w = (ws0_w, ws1_w, ws2_w, ws3_w)
    stage = [_Packed(r, 'val', 'val') for r in stage_w]

    def x_copy(i):
        rows = _rows(i, U * LANES)
        return pltpu.make_async_copy(x_hbm.at[rows], x_v.at[rows], sem_x.at[i])

    def wsp_copy(i):
        rows = _rows(i, U * LANES)
        return pltpu.make_async_copy(wsp_hbm.at[rows], wsp_v.at[rows], sem_sp.at[i])

    def wo_copy(i):
        rows = _rows(i, U * 2 * DH)
        return pltpu.make_async_copy(wo_hbm.at[rows], wo_v.at[rows], sem_wo.at[i])

    def qkv_copies(i):
        cps = []
        for u in range(U):
            j = i * U + u
            for m, w in enumerate((wk_hbm, wq_hbm, wv_hbm)):
                w32 = w.bitcast(U32)
                for b in range(2):
                    cps.append(pltpu.make_async_copy(
                        w32.at[:, b, j, :], wqkv_w.at[6 * j + 3 * b + m], sem_a.at[i]))
        return cps

    def qkv_wait(i):
        filled = wqkv_w.at[_rows(i, 6 * U)]
        pltpu.make_async_copy(filled, filled, sem_a.at[i]).wait()

    w2_copy = pltpu.make_async_copy(wint_hbm.at[pl.ds(FH, FH)], wint_v.at[pl.ds(FH, FH)], sem_w.at[0])
    w1_copy = pltpu.make_async_copy(wint_hbm.at[pl.ds(0, FH)], wint_v.at[pl.ds(0, FH)], sem_w.at[1])
    wout_copy = pltpu.make_async_copy(wout_hbm, wout_v, sem_w.at[2])
    b_copy = pltpu.make_async_copy(b_hbm, b_v, sem_w.at[3])
    mem_copy = pltpu.make_async_copy(mem_hbm, mem_v, sem_w.at[4])
    x0_copy = pltpu.make_async_copy(x_hbm.at[pl.ds(0, LANES)], x0_v, sem_w.at[5])

    x0_copy.start()
    for u in range(zero.shape[0]):
        zero[u] = 0
    w2_copy.start()
    w1_copy.start()
    for i in range(NIT):
        x_copy(i).start()
    for c in (wout_copy, b_copy, mem_copy):
        c.start()

    def timed_after(result):
        if not cfg["pin"]:
            return lambda v: v
        always = jnp.full((8, LANES), zero[31], jnp.int32) == 0

        def after(v):
            r, c = v.shape
            token = pltpu.bitcast(result[:8, :LANES], v.dtype)
            return jnp.where(jnp.tile(always, (r // 8, c // LANES)), v, jnp.tile(token, (r // 8, c // LANES)))

        return after

    def norm(x):
        x = x.astype(F32)
        m = jnp.mean(x, axis=-1, keepdims=True)
        d = x - m
        v = jnp.mean(d * d, axis=-1, keepdims=True)
        return (d * lax.rsqrt(v + EPS)).astype(BF16)

    def fold(z):
        return jnp.sum(z.reshape(z.shape[0] // 8, 8, LANES), axis=0)

    def spread(jobs, n):
        slots = [[] for _ in range(n)]
        total, spent = sum(cost for cost, _ in jobs), 0
        for cost, job in jobs:
            slots[spent * n // total].append(job)
            spent += cost
        return slots

    def in_proj(i, u, starts):
        rc = cfg["rc1"]
        nc = FH // rc
        n = cfg["lnrows"]

        def project(r, slots):
            z = None
            for k in range(NN):
                cols = pl.ds(k * LANES, LANES)
                part = _dot_nt(wint_v[pl.ds(r, rc), cols], stage[u][:, cols])
                z = part if k == 0 else z + part
                for job in slots[k]:
                    job(timed_after(part))
            return z

        def norm_next(r, after):
            rows = pl.ds(pl.multiple_of((i + 1) * LANES + r, n), n)
            x = x_v[rows, :].astype(F32)
            if cfg["lnpin"] & 1:
                x = jnp.concatenate([after(x[:, :LANES]), x[:, LANES:]], axis=1)
            w = pltpu.bitcast(norm(x), U32)
            if cfg["lnpin"] & 2:
                w = after(w)
            xn_w[pl.ds(pl.multiple_of(((i + 1) * LANES + r) // 2, n // 2), n // 2), :] = w
            stage_w[(u + 1) % U][pl.ds(r // 2, n // 2), :] = w

        draw = (d0_v, d1_v)[u % 2]
        lead = cfg["ln1a"]
        slots = [[]] * lead + spread([(1, functools.partial(norm_next, r)) for r in range(0, LANES, n)], nc * NN - lead)
        for c in range(nc):
            z = project(FH + c * rc, slots[c * NN:])
            z = z * (1.0 + _gelu_tanh(z))
            if c == 0:
                shift = jnp.sum(fold(z), axis=0, keepdims=True) * (1.0 / rc)
            d = z - shift
            draw[pl.ds(c * rc, rc), :] = d
            s1 = fold(d) if c == 0 else s1 + fold(d)
            s2 = fold(d * d) if c == 0 else s2 + fold(d * d)
            for e, cp in enumerate(starts):
                if e * nc // len(starts) == c:
                    cp.start()
        mean = jnp.sum(s1, axis=0, keepdims=True) * (1.0 / FH)
        var = jnp.maximum(jnp.sum(s2, axis=0, keepdims=True) * (1.0 / FH) - mean * mean, 0.0)
        inv = lax.rsqrt(var + 4.0 * EPS)

        def rescale(r, after):
            z = (draw[pl.ds(r, 16), :] - mean) * inv
            z2_w[i, pl.ds(r // 2, 8), :] = after(pltpu.bitcast(z.astype(BF16), U32))

        lead = cfg["ln2a"]
        slots = [[]] * lead + spread([(1, functools.partial(rescale, r)) for r in range(0, FH, 16)], nc * NN - lead)
        for c in range(nc):
            z = project(c * rc, slots[c * NN:])
            zt[i, pl.ds(c * rc, rc), :] = (0.5 * z) * (1.0 + _gelu_tanh(z))

    x_v[pl.ds(S, LANES), :] = jnp.zeros((LANES, D), BF16)
    x0_copy.wait()
    for r in range(0, LANES, 32):
        w = pltpu.bitcast(norm(x0_v[pl.ds(r, 32), :]), U32)
        xn_w[pl.ds(r // 2, 16), :] = w
        stage_w[0][pl.ds(r // 2, 16), :] = w
    w2_copy.wait()
    w1_copy.wait()
    x_copy(0).wait()

    def phase1(o, _):
        with jax.named_scope("wait1"):
            @pl.when(o + 1 < NIT)
            def _():
                x_copy(o + 1).wait()

        starts = [wsp_copy(o), wo_copy(o)] + qkv_copies(o)
        for u in range(U):
            in_proj(o * U + u, u, starts[u * len(starts) // U:(u + 1) * len(starts) // U])

    if '1' not in cfg['skip']:
        with jax.named_scope('phase1'):
            lax.fori_loop(0, NIT, phase1, None)
    for c in (wout_copy, b_copy, mem_copy):
        c.wait()
    b32[...] = b_v[...].astype(F32)
    if 't' not in cfg['skip']:
        woutt[...] = wout_v[...].T

    def repack_jobs(j):
        n = cfg["rprows"]

        def qkv(m, r, after):
            rows = pl.ds(r, n)
            t = 6 * j + m
            a = wqkv_w[t, rows, :]
            b = wqkv_w[t + 3, rows, :]
            wqkv_w[t, rows, :] = after((a & U32(0xFFFF)) | (b << 16))
            wqkv_w[t + 3, rows, :] = after((a >> 16) | (b & U32(0xFFFF0000)))

        def out(r, after):
            src = pl.ds(j * (2 * DH) + r, 16)
            dst = pl.ds(j * DH + r // 2, 8)
            wo_w[dst, :] = after(pltpu.bitcast(wo_v[src, :], U32))

        return ([(n, functools.partial(qkv, m, r)) for m in range(3) for r in range(0, D // 2, n)]
                + [(20, functools.partial(out, r)) for r in range(0, 2 * DH, 16)])

    def weight_sum_jobs(load, store):
        def job(r, cluster, members, after):
            words = {}
            for weight, slot in members:
                for _, k, n in weight:
                    if (k, n) not in words:
                        words[k, n] = load(k, n, pl.multiple_of(zero[cluster], 64) + r)
                sums = [_signed_sum([
                    (s, pltpu.unpack_elementwise(words[k, n], index=e, packed_dtype=BF16, unpacked_dtype=F32))
                    for s, k, n in weight]) for e in range(2)]
                store(slot, pl.ds(r, 8), after(pltpu.pack_elementwise(sums, packed_dtype=BF16)))

        return [(sum(3 * len(weight) for weight, _ in members), functools.partial(job, r, cluster, members))
                for r in range(0, DH // 2, 8) for cluster, members in enumerate(clusters)]

    def qkv_sum_jobs(c, m):
        def load(k, n, r):
            return wqkv_w[3 * (h_rest + NB * c + n) + m, pl.ds(r + k * (DH // 2), 8), :]

        def store(slot, rows, w):
            wfq_w[3 * c + m, slot, rows, :] = w

        return weight_sum_jobs(load, store)

    def out_sum_jobs(g):
        def load(k, n, r):
            return wo_w[pl.ds(g * (NB * DH // 2) + r + k * (DH // 2), 8), pl.ds(n * LANES, LANES)]

        def store(slot, rows, w):
            wfo_w[slot, pl.ds(g * (DH // 2) + rows.start, rows.size), :] = w

        return weight_sum_jobs(load, store)

    def stage_jobs(i, dst):
        def job(r, sb, after):
            cols = pl.ds(sb * LANES, LANES)
            dst[pl.ds(r // 2, 8), cols] = after(pltpu.bitcast(wsp_v[pl.ds(i * LANES + r, 16), cols], U32))

        return [(1, functools.partial(job, r, sb)) for sb in range(NTB) for r in range(0, LANES, 16)]

    def mix(i, yt, ws, jobs):
        rc = cfg["rc2"]
        nc = FH // rc
        bias = b32[pl.ds(i, 1), :]
        for c in range(nc):
            rows = pl.ds(c * rc, rc)
            g = bias
            for sb in range(NTB):
                part = _dot_nt(z2[sb, rows, :], ws[:, pl.ds(sb * LANES, LANES)])
                g = g + part
                for job in jobs[c * NTB + sb]:
                    job(timed_after(part))
            yt[rows, :] = (zt[i, rows, :] * g).astype(BF16)
        dc = cfg["dc"]
        for d0 in range(0, D, dc):
            o = _dot(woutt[pl.ds(d0, dc), :], yt[...])
            gate[_rows(i, LANES), pl.ds(d0, dc)] = (o * jax.nn.sigmoid(o)).T

    def phase2(o, _):
        with jax.named_scope("wait2"):
            @pl.when(o + 1 < NIT)
            def _():
                wsp_copy(o + 1).wait()
            wo_copy(o).wait()
            qkv_wait(o)
        jobs = []
        for u in range(U):
            jobs += repack_jobs(o * U + u)[:1 if 'R' in cfg['skip'] else None]
        if cfg["pre"] == "inline":
            assert U == 4
            for e in range(2):
                for m in range(3):
                    jobs += qkv_sum_jobs(jnp.maximum(2 * o - 2 + e, 0), m)
            g0 = (3 * o + 1) // 2 - 1
            for e in range(2):
                jobs += out_sum_jobs(jnp.maximum(g0 + e, 0))
        nc = FH // cfg["rc2"] * NTB
        slots = spread(jobs, U * nc)
        for u in range(U):
            i = o * U + u
            ahead = spread(stage_jobs(jnp.minimum(i + 1, NTB - 1), ws_w[(u + 1) % U]), nc)
            mix(i, yta if u % 2 == 0 else ytb, _Packed(ws_w[u], "val", "val"),
                [a + b for a, b in zip(ahead, slots[u * nc:(u + 1) * nc])])

    wsp_copy(0).wait()
    for _, job in stage_jobs(0, ws_w[0]):
        job(lambda v: v)
    if '2' not in cfg['skip']:
        with jax.named_scope('phase2'):
            lax.fori_loop(0, NIT, phase2, None)
    if cfg["pre"] == "after":
        def q_sums(c, _):
            for m in range(3):
                for _, job in qkv_sum_jobs(c, m):
                    job(lambda v: v)

        def o_sums(g, _):
            for _, job in out_sum_jobs(g):
                job(lambda v: v)

        lax.fori_loop(0, n_fo, q_sums, None)
        lax.fori_loop(0, n_fo, o_sums, None)

    R = 2 * L
    row = lax.broadcasted_iota(jnp.int32, (R, R), 0)
    col = lax.broadcasted_iota(jnp.int32, (R, R), 1)
    rb = (row >= L).astype(jnp.int32)
    cb = (col >= L).astype(jnp.int32)
    ri = row - rb * L
    ci = col - cb * L
    same_head = rb == cb
    keep = same_head & ((ri < M) | (ri >= ci))
    fill = jnp.where(same_head, -1e9 * LOG2E, -jnp.inf).astype(F32)
    scale = DH ** -0.5 * LOG2E
    T = seg - M

    def stack(parts):
        return jnp.concatenate(parts, axis=0)

    def left_sums(block, store):
        base = {}

        def term(b, k):
            if (b, k) not in base:
                if b == "R":
                    base[b, k] = term("P", k) - term("Q", k)
                else:
                    base[b, k] = block(0 if b == "P" else 1, k)
            return base[b, k]

        for r, (left, _, _, _) in enumerate(products):
            store(r, _signed_sum([(s, term(b, k)) for s, b, k in left]).astype(BF16))

    def scatter(acc, out, m):
        for s, b, n in out:
            if (b, n) not in acc:
                acc[b, n] = m if s > 0 else -m
            else:
                acc[b, n] = acc[b, n] + m if s > 0 else acc[b, n] - m

    order = [6 * g + 3 * b + m for g in range(H // 2) for m in range(3) for b in range(2)]
    last_use = [max(r for r, p in enumerate(products) if any(o[2] == n for o in p[2])) for n in range(NB)]

    def four_steps(grp, mem):
        t0 = pl.multiple_of(grp * 4 * seg, 4 * seg)
        mxu = _Stream()

        def tokens(r, n, k):
            return xn[pl.ds(t0 + r, n), pl.ds(k * LANES, LANES)].astype(F32)

        def finish(r, n, k, s):
            rows, cols = pl.ds(t0 + r, n), pl.ds(k * LANES, LANES)
            out_v[rows, cols] = (x_v[rows, cols].astype(F32) + s * gate[rows, cols]).astype(out_v.dtype)

        for j in range(4):
            if 'WXYZ'[j] in cfg['skip']: continue
            tiles = {}
            done = {}

            def attend(g, j=j, tiles=tiles, done=done):
                st = {}

                def scores():
                    q = stack([tiles.pop(6 * g + 1), tiles.pop(6 * g + 4)]).astype(BF16)
                    k = stack([tiles.pop(6 * g), tiles.pop(6 * g + 3)]).astype(BF16)
                    sc = jnp.where(keep, _dot_nt(q, k) * scale, fill)
                    p = jnp.exp2(sc - jnp.max(sc, axis=1, keepdims=True))
                    st["p"] = (p * (1.0 / jnp.sum(p, axis=1, keepdims=True))).astype(BF16)
                    st["t"] = mxu.now + cfg["lat_p"]
                    values_ready()

                def values_ready():
                    if "p" in st and 6 * g + 5 in tiles:
                        mxu.defer(max(st["t"], done["v", g] + cfg["lat_s"]), R // 4, values)

                def values():
                    v = stack([tiles.pop(6 * g + 2), tiles.pop(6 * g + 5)]).astype(BF16)
                    o2 = _dot(st.pop("p"), v)
                    for e in range(2):
                        hd = 2 * g + e
                        o = o2[e * L:(e + 1) * L]
                        parts = [o[:M]] + ([o_carry[hd, pl.ds(0, M * j), :]] if j else [])
                        if j < 3:
                            new = T - M * j
                            o16[:, pl.ds(hd * DH, DH)] = stack(parts + [o[M:M + new]]).astype(BF16)
                            o_carry[hd, pl.ds(0, seg - new), :] = o[M + new:]
                        else:
                            o32[hd] = stack(parts + [o[M:]])
                            if hd % NB == NB - 1:
                                kg = hd // NB

                                def keep_left(r, a, kg=kg):
                                    lo[r, :, pl.ds(kg * DH, DH)] = a

                                left_sums(lambda t, k: o32[NB * kg + k, pl.ds(t * seg, seg), :], keep_left)
                    done["o", g] = mxu.now

                def on_tile(pos):
                    if pos == 4:
                        mxu.defer(mxu.now + cfg["lat_s"], R // 4, scores)
                    elif pos == 5:
                        done["v", g] = mxu.now
                        values_ready()

                return on_tile

            notify = [attend(g) for g in range(H // 2)]

            def tile_done(t, y, j=j, tiles=tiles, notify=notify):
                old = 0 if j == 0 else T - M * (j - 1)
                parts = [y[:M]] + ([qkv_carry[t, pl.ds(0, old), :]] if old else [])
                tiles[t] = stack(parts + [y[M:M + seg - old]])
                if j < 3:
                    qkv_carry[t, pl.ds(0, T - M * j), :] = y[M + seg - old:]
                notify[t // 6](t % 6)

            if j == 0:
                h = [stack([mem[k], tokens(0, 2 * seg, k)[:seg + T]]) for k in range(NN)]
                hh = jnp.concatenate(h, axis=1).astype(BF16)
                for t in order[:3 * h_rest]:
                    tile_done(t, mxu.run(NN * seg // 2, lambda: _dot(hh, wqkv[t])))

                def keep_left(r, a):
                    lq[r] = a

                left_sums(lambda t, k: h[k][t * seg:(t + 1) * seg], keep_left)
                for c in range(n_fo):
                    for m in range(3):
                        t0_ = 3 * (h_rest + NB * c) + m
                        acc = {}
                        for r, (_, weight, out, slot) in enumerate(products):
                            def product():
                                if slot is None:
                                    _, k, n = weight[0]
                                    return _dot(lq[r], wqkv[t0_ + 3 * n, pl.ds(k * LANES, LANES), :])
                                return _dot(lq[r], wfq[3 * c + m, slot])

                            scatter(acc, out, mxu.run(seg // 4, product))
                            for n in range(NB):
                                if last_use[n] == r:
                                    tile_done(t0_ + 3 * n, stack(
                                        [acc["U", n] + acc["S", n], acc["V", n] + acc["S", n]]))
            else:
                r0 = seg + T * j
                a0 = r0 // 16 * 16
                h = [stack([mem[k], tokens(a0, seg, k)[r0 - a0:r0 - a0 + T]]).astype(BF16) for k in range(NN)]
                first = {}
                for k in range(NN):
                    for t in order[:cfg["kfirst"]]:
                        y = mxu.run(seg // 4, lambda: _dot(h[k], wqkv[t, pl.ds(k * LANES, LANES), :]))
                        first[t] = y if k == 0 else first[t] + y
                        if k == NN - 1:
                            tile_done(t, first.pop(t))
                hh = jnp.concatenate(h, axis=1)
                for t in order[cfg["kfirst"]:]:
                    tile_done(t, mxu.run(NN * seg // 4, lambda: _dot(hh, wqkv[t])))

            def need(hd, done=done):
                mxu.until(lambda: ("o", hd // 2) in done)

            if j < 3:
                acc = [None] * NN

                def oproj(hd, n):
                    need(hd)
                    y = mxu.run(seg // 4, lambda: _dot(
                        o16[:, pl.ds(hd * DH, DH)], wo[pl.ds(hd * DH, DH), pl.ds(n * LANES, LANES)]))
                    acc[n] = y if acc[n] is None else acc[n] + y

                for hd in range(H - cfg["hn"]):
                    for n in range(NN):
                        oproj(hd, n)
                for n in range(NN):
                    for hd in range(H - cfg["hn"], H):
                        oproj(hd, n)
                    finish(T * j, T, n, acc[n][M:])
                mem = [a[:M] for a in acc]
            else:
                acc = {}
                for g0, g1 in ((0, cfg["osplit"]), (cfg["osplit"], n_fo)):
                    need(NB * g1 - 1)
                    span = pl.ds(g0 * DH, (g1 - g0) * DH)
                    for r, (_, weight, out, slot) in enumerate(products):
                        def product(r=r, weight=weight, slot=slot):
                            if slot is None:
                                _, k, n = weight[0]
                                w = stack([wo[pl.ds((NB * g + k) * DH, DH), pl.ds(n * LANES, LANES)]
                                           for g in range(g0, g1)])
                            else:
                                w = wfo[slot, span, :]
                            return _dot(lo[r, :, span], w)

                        scatter(acc, out, mxu.run((g1 - g0) * seg // 4, product))
                need(H - 1)
                rest = jnp.concatenate([o32[hd] for hd in range(NB * n_fo, H)], axis=1).astype(BF16)
                mem = []
                for n in range(NN):
                    y = mxu.run((H - NB * n_fo) * seg // 2, lambda: _dot(
                        rest, wo[pl.ds(NB * n_fo * DH, (H - NB * n_fo) * DH), pl.ds(n * LANES, LANES)]))
                    y = y + stack([acc["U", n] + acc["S", n], acc["V", n] + acc["S", n]])
                    finish(3 * T, seg + T, n, y[M:])
                    mem.append(y[:M])
            assert not tiles and not mxu.waiting
        rows = pl.ds(t0, 4 * seg)
        pltpu.make_async_copy(out_v.at[rows], out_hbm.at[rows], sem_o.at[0]).start()
        return mem

    mem0 = mem_v[...].astype(F32)
    if 'a' not in cfg['skip']:
      with jax.named_scope('phaseA'):
        lax.fori_loop(0, S // (4 * seg), four_steps, [mem0[:, n * LANES:(n + 1) * LANES] for n in range(NN)])
    pltpu.make_async_copy(out_v, out_hbm, sem_o.at[0]).wait()


def build(cfg):
    def fn(A_x, A_mem0, A_Wq, A_Wk, A_Wv, A_Wo, A_seg_len, B_x, B_w_in, B_w_sp, B_b_sp, B_w_out):
        del B_x
        B, S, D = A_x.shape
        M = A_mem0.shape[1]
        H, DH = A_Wq.shape[1], A_Wq.shape[2]
        FH = B_w_out.shape[0]
        seg = int(A_seg_len)
        assert B == 1 and DH == LANES
        ntb = S // LANES
        products, slots = _parse_scheme()
        n_fo = H // NB
        vmem = pltpu.VMEM
        dma = pltpu.SemaphoreType.DMA
        scratch = [
            vmem((S + LANES, D), BF16),
            vmem((LANES, D), BF16),
            vmem(((S + LANES) // 2, D), U32),
            *[vmem((LANES // 2, D), U32)] * 4,
            vmem((M, D), BF16),
            vmem((2 * FH, D), BF16),
            vmem((S, S), BF16),
            vmem((FH, D), BF16),
            vmem((D // 2, FH), U32),
            vmem((ntb, LANES), BF16),
            vmem((ntb, LANES), F32),
            vmem((ntb, FH, LANES), F32),
            vmem((FH, LANES), F32),
            vmem((FH, LANES), F32),
            vmem((ntb, FH // 2, LANES), U32),
            *[vmem((LANES // 2, S), U32)] * 4,
            vmem((FH // 2, LANES), U32),
            vmem((FH // 2, LANES), U32),
            vmem((S, D), F32),
            vmem((3 * H, D // 2, DH), U32),
            vmem((H * DH, D), BF16),
            vmem((H * DH // 2, D), U32),
            vmem((3 * n_fo, slots, DH // 2, LANES), U32),
            vmem((slots, n_fo * DH // 2, LANES), U32),
            vmem((len(products), seg // 2, LANES), U32),
            vmem((len(products), seg // 2, n_fo * DH), U32),
            vmem((3 * H, seg - M, DH), F32),
            vmem((H, seg - M, DH), F32),
            vmem((seg // 2, H * DH), U32),
            vmem((H, 2 * seg, DH), F32),
            vmem((S, D), A_x.dtype),
            pltpu.SMEM((32,), jnp.int32),
            dma((ntb,)), dma((6,)), dma((ntb,)), dma((ntb,)), dma((ntb,)), dma((1,)),
        ]
        hbm = pl.BlockSpec(memory_space=pltpu.HBM)
        out = pl.pallas_call(
            functools.partial(_kernel, seg=seg, cfg=cfg),
            out_shape=jax.ShapeDtypeStruct((S, D), A_x.dtype),
            in_specs=[hbm] * 10,
            out_specs=hbm,
            scratch_shapes=scratch,
            compiler_params=pltpu.CompilerParams(
                vmem_limit_bytes=120 * 2**20,
                flags={k: True for k in cfg["flags"].split(",") if k} or None),
        )(
            A_x.reshape(S, D),
            A_mem0.reshape(M, D),
            A_Wq.reshape(D // 2, 2, H, DH),
            A_Wk.reshape(D // 2, 2, H, DH),
            A_Wv.reshape(D // 2, 2, H, DH),
            A_Wo.reshape(H * DH, D),
            B_w_in.T,
            B_w_sp,
            B_b_sp.reshape(ntb, LANES),
            B_w_out,
        )
        return out.reshape(B, S, D)

    return fn


@functools.partial(jax.jit, static_argnames=("A_seg_len",))
def pallas_recurrent_scan__memory_aug_recurrent_mem_tr__mixer_gmlp__prompt_kernel(
    A_x, A_mem0, A_Wq, A_Wk, A_Wv, A_Wo, A_seg_len, B_x, B_w_in, B_w_sp, B_b_sp, B_w_out,
):
    return build(CFG)(A_x, A_mem0, A_Wq, A_Wk, A_Wv, A_Wo, A_seg_len, B_x, B_w_in, B_w_sp, B_b_sp, B_w_out)
```

```python
import functools
import math

import jax
import jax.numpy as jnp
from jax import lax
import jax.experimental.pallas as pl
import jax.experimental.pallas.tpu as pltpu

F32 = jnp.float32
BF16 = jnp.bfloat16
U32 = jnp.uint32
LANES = 128
LOG2E = 1.4426950408889634
EPS = 1e-5

_SCHEME_5 = """
+Q0 | +00 -20 -30 -04 -01 +10 | +S0 | 0
+R0 | +00 -02 -03 -40 +01 -10 | +U0 | 0
+Q1 | +11 -21 -31 -14 +32 | +S1 | 0
+R1 | +11 -12 -13 -41 +23 | +U1 | 0
+R2 | -22 +20 +21 +42 -10 | +V2 | 1
+P2 | +22 -02 -12 -24 +01 | +S2 | 1
+R3 | -33 +30 +31 +43 -32 +23 | +V3 | 1
+P3 | +33 -03 -13 -34 -32 +23 | +S3 | 1
+Q4 | +44 -40 -41 -24 -34 | +V4 | 1
+P4 | +44 -04 -14 -42 -43 | +U4 | 1
+Q0 +Q2 | +20 -10 | +V0 +V2 | 2
+P0 +P2 | +02 -01 | +U0 +U2 | 2
+Q0 +P2 | -02 +20 +01 -10 | +U0 -V2 | 2
+Q0 +Q3 | +30 | +V0 +V3
+P0 +P3 | +03 | +U0 +U3
+Q0 +P3 | -03 +30 | +U0 -V3 | 2
+R0 +R4 | -40 | +V0 +V4
+P0 +P4 | +04 | +S0 +S4
+R0 +P4 | -04 +40 | +S0 +V4 | 2
+R0 +R1 +R2 | -10 | +V0 +V1 +V2
+P0 +P1 +P2 | +01 | +S0 +S1 +S2
+R0 +P1 +P2 | -01 +10 | +S0 +V1 +V2 | 3
+Q1 +Q2 | +21 -10 -32 | +V1 +V2 | 3
+P1 +P2 | +12 -01 -23 | +U1 +U2 | 3
+Q1 +P2 | -12 +21 | +U1 -V2 | 3
+Q3 +Q1 +Q2 | +32 | +S3 +S1 +S2
+R3 +R1 +R2 | +23 | +U3 +U1 +U2
+R3 -Q1 -Q2 | +32 -23 | +S3 +U1 +U2 | 4
+Q1 +Q3 | +31 -32 | +V1 +V3 | 4
+P1 +P3 | +13 -23 | +U1 +U3 | 4
+Q1 +P3 | -13 +31 -32 +23 | +U1 -V3 | 4
+R1 +R4 | -41 | +V1 +V4
+P1 +P4 | +14 | +S1 +S4
+R1 +P4 | -14 +41 | +S1 +V4 | 4
+Q2 +Q4 | +24 | +S2 +S4
+R2 +R4 | +42 | +U2 +U4
+R2 -Q4 | +24 -42 | +S2 +U4 | 4
+Q3 +Q4 | +34 | +S3 +S4
+R3 +R4 | +43 | +U3 +U4
+R3 -Q4 | +34 -43 | +S3 +U4 | 4
"""
_SCHEME_4 = """
+Q0 | +00 -20 -03 -01 +10 | +S0
+R0 | +00 -02 -30 +01 -10 | +U0
+Q0 +Q2 | +20 -10 | +V0 +V2
+P0 +P2 | +02 -01 | +U0 +U2
+Q0 +P2 | -02 +20 +01 -10 | +U0 -V2
+R0 +R3 | -30 | +V0 +V3
+P0 +P3 | +03 | +S0 +S3
+R0 +P3 | -03 +30 | +S0 +V3
+R0 +R1 +R2 | -10 | +V0 +V1 +V2
+P0 +P1 +P2 | +01 | +S0 +S1 +S2
+R0 +P1 +P2 | -01 +10 | +S0 +V1 +V2
+Q1 | +11 -21 -13 | +S1
+R1 | +11 -12 -31 | +U1
+Q1 +Q2 | +21 -10 | +V1 +V2
+P1 +P2 | +12 -01 | +U1 +U2
+Q1 +P2 | -12 +21 | +U1 -V2
+R1 +R3 | -31 | +V1 +V3
+P1 +P3 | +13 | +S1 +S3
+R1 +P3 | -13 +31 | +S1 +V3
+R2 | -22 +20 +21 +32 -10 | +V2
+P2 | +22 -02 -12 -23 +01 | +S2
+Q2 +Q3 | +23 | +S2 +S3
+R2 -Q3 | +23 -32 | +S2 +U3
+R2 +R3 | +32 | +U2 +U3
+Q3 | +33 -30 -31 -23 | +V3
+P3 | +33 -03 -13 -32 | +U3
"""
_SCHEME_2 = """
+Q0 | +00 -10 | +S0
+R0 | +00 -01 | +U0
+P0 +P1 | +01 | +U0 +U1
+Q0 +P1 | -01 +10 | +U0 -V1
+Q0 +Q1 | +10 | +V0 +V1
+P1 | +11 -01 | +S1
+R1 | -11 +10 | +V1
"""

IN_ROWS = 96
IN_ARRIVAL = (2, 4, 6)
MIX_ROWS = 144
SCORE_DELAY = 260
VALUE_DELAY = 700


def _parse_scheme(text):
    sign = {"+": 1, "-": -1}
    products, groups = [], {}
    for line in text.strip().split("\n"):
        left, weight, out, *group = (part.split() for part in line.split("|"))
        left = [(sign[t[0]], t[1], int(t[2])) for t in left]
        weight = [(sign[t[0]], int(t[1]), int(t[2])) for t in weight]
        out = [(sign[t[0]], t[1], int(t[2])) for t in out]
        if len(weight) == 1:
            out = [(s * weight[0][0], b, n) for s, b, n in out]
            products.append((left, [(1,) + weight[0][1:]], out, None))
        else:
            slot = sum(len(g) for g in groups.values())
            products.append((left, sorted(weight, reverse=True), out, slot))
            groups.setdefault(str(group), []).append((products[-1][1], slot))
    return products, [groups[g] for g in sorted(groups)]


def _signed_sum(terms):
    terms = sorted(terms, key=lambda t: -t[0])
    total = terms[0][1] if terms[0][0] > 0 else -terms[0][1]
    for s, v in terms[1:]:
        total = total + v if s > 0 else total - v
    return total


def _left_terms(left):
    return [(s * t, half, k) for s, b, k in left
            for t, half in {"P": [(1, 0)], "Q": [(1, 1)], "R": [(1, 0), (-1, 1)]}[b]]


def _scatter(acc, out, m):
    for s, b, n in out:
        if (b, n) not in acc:
            acc[b, n] = m if s > 0 else -m
        else:
            acc[b, n] = acc[b, n] + m if s > 0 else acc[b, n] - m


def _fast_matmul(scheme, product, direct, emit):
    acc = {}
    blocks = max(o[2] for p in scheme for o in p[2]) + 1
    last = {(half, n): max(r for r, p in enumerate(scheme) if any(o[1:] in (("UV"[half], n), ("S", n)) for o in p[2]))
            for half in range(2) for n in range(blocks)}
    for r, (_, _, out, _) in enumerate(scheme):
        _scatter(acc, out, product(r))
        for (half, n), when in last.items():
            if when == r:
                total = acc["UV"[half], n] + acc["S", n]
                emit(half, n, total if direct is None else total + direct(half, n))


def _dot(a, b):
    return jnp.dot(a, b, preferred_element_type=F32)


def _dot_nt(a, b):
    return lax.dot_general(a, b, (((1,), (1,)), ((), ())), preferred_element_type=F32)


def _stack(parts):
    return jnp.concatenate(parts, axis=0)


def _rows(i, n):
    if isinstance(i, int):
        return pl.ds(i * n, n)
    return pl.ds(pl.multiple_of(i * n, n), n)


def _words(x):
    return pltpu.bitcast(x.astype(BF16), U32)


def _zip_rows(x):
    return _stack([pltpu.pack_elementwise([x[r:r + 8], x[r + 8:r + 16]], packed_dtype=BF16)
                   for r in range(0, x.shape[0], 16)])


def _word_sum(terms):
    if len(terms) == 1 and terms[0][0] > 0:
        return terms[0][1]
    return pltpu.pack_elementwise(
        [_signed_sum([(s, pltpu.unpack_elementwise(w, index=e, packed_dtype=BF16, unpacked_dtype=F32))
                      for s, w in terms]) for e in range(2)], packed_dtype=BF16)


class _Packed:
    def __init__(self, words):
        self.words = words

    def __getitem__(self, idx):
        idx = idx if isinstance(idx, tuple) else (idx,)
        at = len(self.words.shape) - 2
        if len(idx) > at and not isinstance(idx[at], slice):
            start = idx[at].start // 2
            if not isinstance(start, int):
                start = pl.multiple_of(start, 8)
            idx = idx[:at] + (pl.ds(start, idx[at].size // 2),) + idx[at + 1:]
        return pltpu.bitcast(self.words[idx], BF16)


def _spread(jobs, n):
    slots = [[] for _ in range(n)]
    total, spent = max(1, sum(cost for cost, _ in jobs)), 0
    for cost, job in jobs:
        slots[spent * n // total].append(job)
        spent += cost
    return slots


def _at_once(jobs):
    for _, job in jobs:
        job(lambda v: v)


class _Stream:
    def __init__(self):
        self.now = 0
        self.waiting = []

    def defer(self, ready, cost, fn):
        self.waiting.append((ready, cost, fn))
        self.waiting.sort(key=lambda w: w[0])

    def _emit_next(self):
        ready, cost, fn = self.waiting.pop(0)
        self.now = max(self.now, ready) + cost
        fn()

    def run(self, cost, fn):
        while self.waiting and self.waiting[0][0] <= self.now:
            self._emit_next()
        self.now += cost
        return fn()

    def until(self, done):
        while not done():
            self._emit_next()


def _kernel(
    x_hbm, mem_hbm, wq_hbm, wk_hbm, wv_hbm, wo_hbm, wint_hbm, wsp_hbm, b_hbm, wout_hbm,
    out_hbm,
    x_v, lna_v, lnb_v, xn_w, xa_w, xb_w, mem_v, wint_w, win_w, wsp_w, wout_v, woutt_w, wol_w, b_v, bias_v,
    z1_v, d_v, z2_w, ws_w, ya_w, yb_w, gate_v, wqkv_w, wo_w, wfq_w, wfo_w,
    lq_w, lo_w, qkv_carry, o_carry, o16_w, o32_v, out_v, zero,
    sem_x, sem_in, sem_small, sem_sp, sem_qkv, sem_wo, sem_out,
    *, seg,
):
    S, D = out_v.shape
    M = mem_v.shape[0]
    H = o_carry.shape[0]
    DH = LANES
    FH = wout_v.shape[0]
    HF = FH // 2
    NTB = S // LANES
    NQ = NTB // 4
    NN = D // LANES
    assert (M, seg, NN, H, NQ) == (8, 32, 5, 32, 4)
    scheme5, sum_groups = _parse_scheme(_SCHEME_5)
    scheme4, _ = _parse_scheme(_SCHEME_4)
    scheme2, _ = _parse_scheme(_SCHEME_2)
    n2 = len(scheme2)
    n_five = H // NN
    xn, xa, xb, win, woutt, wol, z2, ws, ya, yb, wo, wfq, wfo, lq, lo, o16 = map(_Packed, (
        xn_w, xa_w, xb_w, win_w, woutt_w, wol_w, z2_w, ws_w, ya_w, yb_w, wo_w, wfq_w, wfo_w, lq_w, lo_w, o16_w))

    def x_copy(i):
        r0, r1 = (2 * i, 2 * i + 2) if i < 2 else (4 * i - 4, 4 * i)
        rows = pl.ds(r0 * LANES, (r1 - r0) * LANES)
        return pltpu.make_async_copy(x_hbm.at[rows], x_v.at[rows], sem_x.at[i])

    cuts = [0] + [c * IN_ROWS for c in IN_ARRIVAL] + [FH]

    def win_copies(c):
        rows = [pl.ds((half * FH + cuts[c]) // 2, (cuts[c + 1] - cuts[c]) // 2) for half in range(2)]
        return [pltpu.make_async_copy(wint_hbm.bitcast(U32).at[r], wint_w.at[r], sem_in.at[c]) for r in rows]

    def wsp_copy(i):
        rows = _rows(i, 2 * LANES)
        return pltpu.make_async_copy(wsp_hbm.bitcast(U32).at[rows], wsp_w.at[rows], sem_sp.at[i])

    chunks = [range(NN * i, min(NN * (i + 1), H // 2)) for i in range(NQ)]

    def wo_copy(i):
        rows = pl.ds(chunks[i][0] * DH, len(chunks[i]) * DH)
        return pltpu.make_async_copy(wo_hbm.bitcast(U32).at[rows], wo_w.at[rows], sem_wo.at[i])

    def start_attention_weights(i):
        wo_copy(i).start()
        for j in chunks[i]:
            for m, w in enumerate((wk_hbm, wq_hbm, wv_hbm)):
                for b in range(2):
                    pltpu.make_async_copy(
                        w.bitcast(U32).at[:, b, j, :], wqkv_w.at[6 * j + 3 * b + m], sem_qkv.at[i]).start()

    def wait_attention_weights(i):
        wo_copy(i).wait()
        filled = wqkv_w.at[pl.ds(6 * chunks[i][0], 6 * len(chunks[i]))]
        pltpu.make_async_copy(filled, filled, sem_qkv.at[i]).wait()

    small_copies = [pltpu.make_async_copy(src, dst, sem_small.at[0])
                    for src, dst in ((wout_hbm, wout_v), (b_hbm, b_v), (mem_hbm, mem_v))]

    for e in range(zero.shape[0]):
        zero[e] = 0
    x_copy(0).start()
    for c in range(len(cuts) - 1):
        for cp in win_copies(c):
            cp.start()
    x_copy(1).start()

    def timed_after(result):
        always = jnp.full((8, LANES), zero[zero.shape[0] - 1], jnp.int32) == 0

        def after(v):
            reps = (v.shape[0] // 8, v.shape[1] // LANES)
            token = pltpu.bitcast(result[:8, :LANES], v.dtype)
            return jnp.where(jnp.tile(always, reps), v, jnp.tile(token, reps))

        return after

    def run_jobs(groups, result):
        jobs = [job for group in groups for job in group]
        if jobs:
            after = timed_after(result)
            for job in jobs:
                job(after)

    KX = (NN - 1) // 2 * LANES

    def norm_jobs(p, dst_w, ln_v):
        def rows(r, e):
            start = p * (2 * LANES) + pl.multiple_of(zero[e], 64) + r
            return x_v[pl.ds(start, 16), :].astype(F32)

        def mean(r, after):
            ln_v[0, pl.ds(r, 16), :] = after(jnp.broadcast_to(
                jnp.mean(rows(r, 0), axis=-1, keepdims=True), (16, LANES)))

        def centred(r, e):
            return rows(r, e) - jnp.tile(ln_v[0, pl.ds(r, 16), :], (1, NN))

        def scale(r, after):
            d = centred(r, 1)
            ln_v[1, pl.ds(r, 16), :] = after(jnp.broadcast_to(
                lax.rsqrt(jnp.mean(d * d, axis=-1, keepdims=True) + EPS), (16, LANES)))

        def apply(r, after):
            xn_w[pl.ds(p * LANES + r // 2, 8), :] = after(
                _words(centred(r, 2) * jnp.tile(ln_v[1, pl.ds(r, 16), :], (1, NN))))

        def operands(r, after):
            start = p * LANES + pl.multiple_of(zero[3], 64)
            w = [xn_w[pl.ds(start + (n * LANES + r) // 2, 8), :] for n in range(2)]
            for n in range(2):
                dst_w[pl.ds(r // 2, 8), pl.ds(n2 * KX + n * LANES, LANES)] = after(w[n][:, 2 * KX:])
            for e, (_, weight, _, _) in enumerate(scheme2):
                dst_w[pl.ds(r // 2, 8), pl.ds(e * KX, KX)] = after(_word_sum(
                    [(s, w[n][:, k * KX:(k + 1) * KX]) for s, k, n in weight]))

        both = range(0, 2 * LANES, 16)
        return ([(2, functools.partial(mean, r)) for r in both] + [(3, functools.partial(scale, r)) for r in both]
                + [(4, functools.partial(apply, r)) for r in both]
                + [(6, functools.partial(operands, r)) for r in range(0, LANES, 16)])

    def fold(z):
        return jnp.sum(z.reshape(z.shape[0] // 8, 8, LANES), axis=0)

    def in_proj(p, src, early=(), late=(), steady=(), before=lambda c: None, hold=0):
        n_chunks = FH // IN_ROWS
        per = n2 * (KX // LANES) + 4
        slots = iter(zip(*[[[]] * a + _spread(jobs, n_chunks * per - a - b) + [[]] * b
                           for jobs, a, b in ((early, hold * per, 10), (late, 40, 0), (steady, 0, 0))]))
        shift, s1, s2 = {}, {}, {}
        for c in range(n_chunks):
            rows = pl.ds(c * IN_ROWS, IN_ROWS)
            before(c)

            def tile(lhs, rhs):
                part = _dot_nt(win[rows, pl.ds(lhs, LANES)], src[:, pl.ds(rhs, LANES)])
                run_jobs(next(slots), part)
                return part

            def product(r):
                return _signed_sum([(1, tile(r * KX + k, r * KX + k)) for k in range(0, KX, LANES)])

            def direct(half, n):
                return tile(n2 * KX + half * LANES, n2 * KX + n * LANES)

            def emit(half, n, z):
                c0 = math.sqrt(2.0 / math.pi)
                z = z * (1.0 + jnp.tanh(z * (c0 + (c0 * 0.044715) * (z * z))))
                if half == 0:
                    z1_v[2 * p + n, rows, :] = z
                    return
                if c == 0:
                    shift[n] = z[:8]
                d = z - jnp.tile(shift[n], (IN_ROWS // 8, 1))
                d_v[2 * p + n, rows, :] = d
                s1[n] = fold(d) if c == 0 else s1[n] + fold(d)
                s2[n] = fold(d * d) if c == 0 else s2[n] + fold(d * d)

            _fast_matmul(scheme2, product, direct, emit)
        stats = []
        for n in range(2):
            off = jnp.sum(s1[n] + (FH // 8) * shift[n], axis=0, keepdims=True) * (1.0 / FH) - shift[n]
            var = jnp.sum(s2[n] - off * (2.0 * s1[n] - (FH // 8) * off), axis=0, keepdims=True) * (1.0 / FH)
            stats.append((off, 0.25 * lax.rsqrt(jnp.maximum(var, 0.0) + 4.0 * EPS)))
        return stats

    def rescale_jobs(q, stats, timed_input=False):
        def job(r, after):
            off = [jnp.tile(after(stats[n][0]) if timed_input else stats[n][0], (2, 1)) for n in range(4)]
            base = {}
            for k in range(4):
                for half in range(2):
                    base["PQ"[half], k] = (d_v[4 * q + k, pl.ds(half * HF + r, 16), :] - off[k]) * stats[k][1]
                base["R", k] = base["P", k] - base["Q", k]
            for e, (left, _, _, _) in enumerate(scheme4):
                w = _zip_rows(_signed_sum([(s, base[b, k]) for s, b, k in left]))
                z2_w[q, e, pl.ds(r // 2, 8), :] = w if timed_input else after(w)
            return w

        return [(1, functools.partial(job, r)) for r in range(0, HF, 16)]

    def weights_arrived(c):
        for cp in win_copies(c):
            cp.wait()
        if c == len(cuts) - 3:
            for i in range(2, NQ + 1):
                x_copy(i).start()
            for cp in small_copies:
                cp.start()
        if c == len(cuts) - 2:
            wsp_copy(0).start()
            wsp_copy(1).start()
            start_attention_weights(0)
            start_attention_weights(1)
        for r in range(cuts[c], cuts[c + 1], 16):
            w = [wint_w[pl.ds((half * FH + r) // 2, 8), :] for half in range(2)]
            w[0] = _zip_rows(pltpu.bitcast(w[0], BF16).astype(F32))
            for e, (left, _, _, _) in enumerate(scheme2):
                win_w[pl.ds(r // 2, 8), pl.ds(e * KX, KX)] = _word_sum(
                    [(s, w[half][:, k * KX:(k + 1) * KX]) for s, half, k in _left_terms(left)])
            for half in range(2):
                win_w[pl.ds(r // 2, 8), pl.ds(n2 * KX + half * LANES, LANES)] = w[half][:, 2 * KX:]

    KY = HF // LANES * LANES
    DC = LANES // 2
    d_chunks = [(d, 2 * LANES + d) for d in range(0, 2 * LANES, DC)] + [(4 * LANES, 4 * LANES + DC)]

    def out_weight_jobs():
        def hidden_order(r, n, d):
            w = wout_v[pl.ds(r, n), pl.ds(d, LANES)]
            for _ in range(2):
                w = pltpu.bitcast(_zip_rows(w.astype(F32)), BF16)
            return w

        def transpose(col, d, after):
            if col < 2 * KY:
                w = hidden_order(col // KY * HF + col % KY, LANES, d)
            else:
                w = _stack([hidden_order(k * HF + KY, HF - KY, d) for k in range(2)])
            w = pltpu.bitcast(after(pltpu.bitcast(w, U32)), BF16)
            woutt_w[pl.ds(d // 2, LANES // 2), pl.ds(col, w.shape[0])] = pltpu.bitcast(w.T, U32)

        def operands(c, r, after):
            w = [woutt_w[pl.ds((d + r) // 2, 8), pl.ds(0, 2 * KY)] for d in d_chunks[c]]
            for e, (left, _, _, _) in enumerate(scheme2):
                wol_w[pl.ds((c * DC + r) // 2, 8), pl.ds(e * KY, KY)] = after(_word_sum(
                    [(s, w[half][:, k * KY:(k + 1) * KY]) for s, half, k in _left_terms(left)]))

        return ([(2, functools.partial(transpose, col, d)) for d in range(0, D, LANES) for col in range(0, FH, LANES)]
                + [(4, functools.partial(operands, c, r)) for c in range(len(d_chunks)) for r in range(0, DC, 16)])

    def stage_jobs(o):
        def job(r, q, after):
            w = {(k, n): wsp_w[pl.ds(o * (2 * LANES) + (n * LANES + r) // 2, 8), pl.ds((4 * q + k) * LANES, LANES)]
                 for k in range(4) for n in range(4)}
            for e, (_, weight, _, _) in enumerate(scheme4):
                ws_w[e, pl.ds(r // 2, 8), pl.ds(q * LANES, LANES)] = after(_word_sum(
                    [(s, w[k, n]) for s, k, n in weight]))

        return [(1, functools.partial(job, r, q)) for q in range(NQ) for r in range(0, LANES, 16)]

    x_copy(0).wait()
    for r in range(0, 2 * LANES, 16):
        x = x_v[pl.ds(r, 16), :].astype(F32)
        d = x - jnp.mean(x, axis=-1, keepdims=True)
        xn_w[pl.ds(r // 2, 8), :] = _words(d * lax.rsqrt(jnp.mean(d * d, axis=-1, keepdims=True) + EPS))
    _at_once(norm_jobs(0, xa_w, lna_v)[-LANES // 16:])

    def before(c):
        if c * IN_ROWS in cuts:
            weights_arrived(cuts.index(c * IN_ROWS))
        if c == IN_ARRIVAL[-1]:
            x_copy(1).wait()

    stats = in_proj(0, xa, early=norm_jobs(1, xb_w, lna_v), before=before, hold=IN_ARRIVAL[-1])

    def phase1(o, stats):
        for k in range(NQ - 1):
            @pl.when(o == k)
            def _():
                x_copy(k + 2).wait()

        ahead = norm_jobs(2 * o + 3, xb_w, lnb_v)
        odd = in_proj(2 * o + 1, xb, early=norm_jobs(2 * o + 2, xa_w, lna_v), steady=ahead[:32])
        return in_proj(2 * o + 2, xa, late=rescale_jobs(o, stats + odd), steady=ahead[32:])

    stats = lax.fori_loop(0, NQ - 1, phase1, stats)
    for cp in small_copies + [wsp_copy(0)]:
        cp.wait()
    for i in range(2, NQ):
        wsp_copy(i).start()
    start_attention_weights(2)
    stats = stats + in_proj(NTB // 2 - 1, xb, early=out_weight_jobs(), steady=stage_jobs(0))
    results = []
    for _, job in rescale_jobs(NQ - 1, stats, timed_input=True):
        results.append(job(timed_after(results[-2]) if len(results) >= 2 else (lambda v: v)))
    bias_v[...] = 0.25 * b_v[...].astype(F32)

    def repack_jobs(j):
        def job(m, r, after):
            t, rows = 6 * j + m, pl.ds(r, 8)
            a = wqkv_w[t, rows, :]
            b = wqkv_w[t + 3, rows, :]
            wqkv_w[t, rows, :] = after((a & U32(0xFFFF)) | (b << 16))
            wqkv_w[t + 3, rows, :] = after((a >> 16) | (b & U32(0xFFFF0000)))

        return [(16, functools.partial(job, m, r)) for m in range(3) for r in range(0, D // 2, 8)]

    def weight_sum_jobs(load, store, r):
        def job(e, members, after):
            words = {}
            for weight, slot in members:
                for _, k, n in weight:
                    if (k, n) not in words:
                        words[k, n] = load(k, n, pl.multiple_of(r + zero[e], 8))
                store(slot, pl.multiple_of(r, 8), after(_word_sum([(s, words[k, n]) for s, k, n in weight])))

        return [(sum(3 * len(weight) for weight, _ in members), functools.partial(job, e, members))
                for e, members in enumerate(sum_groups)]

    def qkv_sum_jobs(g, m, row):
        def load(k, n, r):
            return wqkv_w[3 * (NN * g + n) + m, pl.ds(r + k * (DH // 2), 8), :]

        def store(slot, r, w):
            wfq_w[3 * g + m, slot, pl.ds(r, 8), :] = w

        return weight_sum_jobs(load, store, row)

    def out_sum_jobs(g, row):
        def load(k, n, r):
            return wo_w[pl.ds(g * (NN * DH // 2) + r + k * (DH // 2), 8), pl.ds(n * LANES, LANES)]

        def store(slot, r, w):
            wfo_w[slot, pl.ds(g * (DH // 2) + r, 8), :] = w

        return weight_sum_jobs(load, store, row)

    def mix(o, jobs):
        rc = MIX_ROWS
        slots = iter(_spread(jobs, HF // rc * len(scheme4) * NQ))
        for c in range(HF // rc):
            ys = {}

            def product(r):
                total = None
                for q in range(NQ):
                    part = _dot_nt(z2[q, r, pl.ds(c * rc, rc), :], ws[r, :, pl.ds(q * LANES, LANES)])
                    total = part if q == 0 else total + part
                    run_jobs([next(slots)], part)
                return total

            def emit(half, n, g):
                ys[half, n] = z1_v[4 * o + n, pl.ds(half * HF + c * rc, rc), :] * (g + bias_v[pl.ds(4 * o + n, 1), :])
                u = n // 2
                if not all((k, 2 * u + t) in ys for k in range(2) for t in range(2)):
                    return
                y_w = (ya_w, yb_w)[u]
                m = max(0, min(rc, KY - c * rc))
                if m:
                    for e, (_, weight, _, _) in enumerate(scheme2):
                        y_w[pl.ds(c * rc // 2, m // 2), pl.ds(e * LANES, LANES)] = _zip_rows(_signed_sum(
                            [(s, ys[k, 2 * u + t][:m]) for s, k, t in weight]))
                if m < rc:
                    for k in range(2):
                        for t in range(2):
                            y_w[pl.ds((k * (HF - KY) + c * rc + m - KY) // 2, (rc - m) // 2),
                                pl.ds((n2 + t) * LANES, LANES)] = _zip_rows(ys[k, 2 * u + t][m:])

            _fast_matmul(scheme4, product, None, emit)

    def out_proj(p, y, jobs):
        slots = iter(_spread(jobs, len(d_chunks) * n2))
        tiles = {}
        for c, d0 in enumerate(d_chunks):
            def part(r, k0, k1):
                total = _dot(wol[pl.ds(c * DC, DC), pl.ds(r * KY + k0, k1 - k0)],
                             y[pl.ds(k0, k1 - k0), pl.ds(r * LANES, LANES)])
                if k1 == KY:
                    run_jobs([next(slots)], total)
                return total

            early = [part(r, 0, KY - LANES) for r in range(3)] if c == 0 else []

            def product(r):
                return early[r] + part(r, KY - LANES, KY) if r < len(early) else part(r, 0, KY)

            def direct(half, n):
                return _dot(woutt[pl.ds(d0[half], DC), pl.ds(2 * KY, FH - 2 * KY)],
                            y[pl.ds(0, FH - 2 * KY), pl.ds((n2 + n) * LANES, LANES)])

            def emit(half, n, h):
                d = d0[half] // LANES * LANES
                done = tiles.setdefault((d, n), {})
                done[d0[half]] = h + h * jnp.tanh(h)
                if len(done) * DC == LANES:
                    gate_v[_rows(2 * p + n, LANES), pl.ds(d, LANES)] = _stack([done[k] for k in sorted(done)]).T

            _fast_matmul(scheme2, product, direct, emit)

    def phase2(o, _):
        for k in range(NQ):
            @pl.when(o == k)
            def _():
                if k + 1 < NQ:
                    wsp_copy(k + 1).wait()
                wait_attention_weights(k)
                if k == 1:
                    start_attention_weights(3)

        whole, shared, row = (3 * o + 1) // 2, o // 2 * 3 + 1, o % 2 * (DH // 4)
        first = [job for r in range(0, DH // 2, 8) for job in out_sum_jobs(whole, r)]
        repack = [job for u in range(NN) for job in repack_jobs(jnp.minimum(o * NN + u, H // 2) if u else o * NN)]
        jobs = [job for a, b in zip(first, _spread([(1, job) for job in repack], len(first))) for job in [a] + b]
        for m in range(3):
            for r in range(0, DH // 2, 8):
                jobs += qkv_sum_jobs(whole, m, r)
            for r in range(0, DH // 4, 8):
                jobs += qkv_sum_jobs(shared, m, row + r)
        for r in range(0, DH // 4, 8):
            jobs += out_sum_jobs(shared, row + r)
        mix(o, jobs)
        ahead = _spread([(1, job) for job in stage_jobs(jnp.minimum(o + 1, NQ - 1))], 2)
        out_proj(2 * o, ya, ahead[0])
        out_proj(2 * o + 1, yb, ahead[1])

    lax.fori_loop(0, NQ, phase2, None)

    L = M + seg
    T = seg - M
    row = lax.broadcasted_iota(jnp.int32, (L, L), 0)
    col = lax.broadcasted_iota(jnp.int32, (L, L), 1)
    keep = (row < M) | (row >= col)
    heads = list(range(NN * n_five, H)) + list(range(NN * n_five))
    order = [3 * (hd + b) + m for hd in heads[::2] for m in range(3) for b in range(2)]
    last_use = [max(r for r, p in enumerate(scheme5) if any(o[2] == n for o in p[2])) for n in range(NN)]

    def left_sum_jobs(block, store):
        base = {}

        def term(b, k):
            if (b, k) not in base:
                base[b, k] = term("P", k) - term("Q", k) if b == "R" else block("PQ".index(b), k)
            return base[b, k]

        def job(r, left, after):
            store(r, after(_words(_signed_sum([(s, term(b, k)) for s, b, k in left]))))

        return [(1, functools.partial(job, r, left)) for r, (left, _, _, _) in enumerate(scheme5)]

    def gather(acc, n):
        return _stack([acc["U", n] + acc["S", n], acc["V", n] + acc["S", n]])

    def four_segments(grp, mem):
        t0 = pl.multiple_of(grp * 4 * seg, 4 * seg)
        mxu = _Stream()

        def tokens(r, n, k):
            return xn[pl.ds(t0 + r, n), pl.ds(k * LANES, LANES)].astype(F32)

        def finish(r, n, k, s):
            rows, cols = pl.ds(t0 + r, n), pl.ds(k * LANES, LANES)
            out_v[rows, cols] = (x_v[rows, cols].astype(F32) + s * gate_v[rows, cols]).astype(out_v.dtype)

        for j in range(4):
            tiles = {}
            done = {}

            def attend(hd, j=j, tiles=tiles, done=done):
                st = {}

                def scores():
                    sc = _dot_nt(tiles.pop(3 * hd + 1), tiles.pop(3 * hd).astype(BF16))
                    sc = jnp.where(keep, sc * (DH ** -0.5 * LOG2E), -1e9 * LOG2E)
                    p = jnp.exp2(sc - jnp.max(sc, axis=1, keepdims=True))
                    st["p"] = p * pl.reciprocal(jnp.sum(p, axis=1, keepdims=True), approx=False, full_range=False)
                    st["t"] = mxu.now + VALUE_DELAY
                    values_ready()

                def values_ready():
                    if "p" in st and 3 * hd + 2 in tiles:
                        mxu.defer(max(st["t"], done["v", hd] + SCORE_DELAY), L // 4, values)

                def values():
                    o = _dot(st.pop("p"), tiles.pop(3 * hd + 2).astype(BF16))
                    parts = [o[:M]] + ([o_carry[hd, pl.ds(0, M * j), :]] if j else [])
                    if j < 3:
                        new = T - M * j
                        o16_w[:, pl.ds(hd * DH, DH)] = _words(_stack(parts + [o[M:M + new]]))
                        o_carry[hd, pl.ds(0, seg - new), :] = o[M + new:]
                    else:
                        o32_v[hd] = _stack(parts + [o[M:]])
                    done["o", hd] = mxu.now
                    g = hd // NN
                    if j == 3 and g < n_five and all(("o", NN * g + k) in done for k in range(NN)):
                        def keep_left(r, a):
                            lo_w[r, :, pl.ds(g * DH, DH)] = a

                        _at_once(left_sum_jobs(lambda t, k: o32_v[NN * g + k, pl.ds(t * seg, seg), :], keep_left))

                def on_tile(m):
                    if m == 1:
                        mxu.defer(mxu.now + SCORE_DELAY, L // 4, scores)
                    elif m == 2:
                        done["v", hd] = mxu.now
                        values_ready()

                return on_tile

            notify = [attend(hd) for hd in range(H)]

            def tile_done(t, y, j=j, tiles=tiles, notify=notify):
                old = 0 if j == 0 else T - M * (j - 1)
                parts = [y[:M]] + ([qkv_carry[t, pl.ds(0, old), :]] if old else [])
                tiles[t] = _stack(parts + [y[M:M + seg - old]])
                if j < 3:
                    qkv_carry[t, pl.ds(0, T - M * j), :] = y[M + seg - old:]
                notify[t // 3](t % 3)

            def need(hds, done=done):
                mxu.until(lambda: all(("o", hd) in done for hd in hds))

            if j == 0:
                h = [_stack([mem[k], tokens(0, 2 * seg, k)[:seg + T]]) for k in range(NN)]
                hh = jnp.concatenate(h, axis=1).astype(BF16)

                def keep_left(r, a):
                    lq_w[r] = a

                plain = order[:3 * (H - NN * n_five)]
                slots = iter(_spread(left_sum_jobs(lambda t, k: h[k][t * seg:(t + 1) * seg], keep_left),
                                     len(plain) * (NN - 1)) + [[]] * len(plain))
                for t in plain:
                    for k in range(NN):
                        part = mxu.run(seg // 2, lambda: _dot(
                            hh[:, k * LANES:(k + 1) * LANES],
                            pltpu.bitcast(wqkv_w[t, _rows(k, DH // 2), :], BF16)))
                        y = part if k == 0 else y + part
                        run_jobs([next(slots)], part)
                    tile_done(t, y)
                for g in range(n_five):
                    for m in range(3):
                        first = 3 * NN * g + m
                        acc = {}
                        for r, (_, weight, out, slot) in enumerate(scheme5):
                            def product():
                                if slot is None:
                                    _, k, n = weight[0]
                                    w = pltpu.bitcast(wqkv_w[first + 3 * n, _rows(k, DH // 2), :], BF16)
                                else:
                                    w = wfq[3 * g + m, slot]
                                return _dot(lq[r], w)

                            _scatter(acc, out, mxu.run(seg // 4, product))
                            for n in range(NN):
                                if last_use[n] == r:
                                    tile_done(first + 3 * n, gather(acc, n))
            else:
                r0 = seg + T * j
                a0 = r0 // 16 * 16
                h = [_stack([mem[k], tokens(a0, seg, k)[r0 - a0:r0 - a0 + T]]).astype(BF16) for k in range(NN)]
                partial = {}
                for k in range(NN):
                    for t in order[:8]:
                        y = mxu.run(seg // 4, lambda: _dot(
                            h[k], pltpu.bitcast(wqkv_w[t, _rows(k, DH // 2), :], BF16)))
                        partial[t] = y if k == 0 else partial[t] + y
                        if k == NN - 1:
                            tile_done(t, partial.pop(t))
                hh = jnp.concatenate(h, axis=1)
                for t in order[8:]:
                    tile_done(t, mxu.run(NN * seg // 4, lambda: _dot(hh, pltpu.bitcast(wqkv_w[t], BF16))))

            if j < 3:
                total = [None] * NN

                def project(hd, n):
                    need([hd])
                    y = mxu.run(seg // 4, lambda: _dot(
                        o16[:, pl.ds(hd * DH, DH)], wo[pl.ds(hd * DH, DH), pl.ds(n * LANES, LANES)]))
                    total[n] = y if total[n] is None else total[n] + y

                for hd in heads[:-8]:
                    for n in range(NN):
                        project(hd, n)
                for n in range(NN):
                    for hd in heads[-8:]:
                        project(hd, n)
                    finish(T * j, T, n, total[n][M:])
                mem = [a[:M] for a in total]
            else:
                acc = {}
                mem = [None] * NN
                rest = range(NN * n_five, H)
                need(rest)
                o_rest = jnp.concatenate([o32_v[hd] for hd in rest], axis=1).astype(BF16)
                for n in range(NN):
                    y = mxu.run(len(rest) * seg // 2, lambda: _dot(
                        o_rest, wo[pl.ds(rest[0] * DH, len(rest) * DH), pl.ds(n * LANES, LANES)]))
                    _scatter(acc, [(1, "U", n)], y[:seg])
                    _scatter(acc, [(1, "V", n)], y[seg:])
                for g0, g1 in ((0, n_five // 2), (n_five // 2, n_five)):
                    need(range(NN * g0, NN * g1))
                    span = pl.ds(g0 * DH, (g1 - g0) * DH)
                    for r, (_, weight, out, slot) in enumerate(scheme5):
                        def product():
                            if slot is None:
                                _, k, n = weight[0]
                                w = _stack([wo[pl.ds((NN * g + k) * DH, DH), pl.ds(n * LANES, LANES)]
                                            for g in range(g0, g1)])
                            else:
                                w = wfo[slot, span, :]
                            return _dot(lo[r, :, span], w)

                        _scatter(acc, out, mxu.run((g1 - g0) * seg // 4, product))
                        for n in range(NN):
                            if g1 == n_five and last_use[n] == r:
                                y = gather(acc, n)
                                finish(3 * T, seg + T, n, y[M:])
                                mem[n] = y[:M]
            assert not tiles and not mxu.waiting
            if j >= 2:
                rows = pl.ds(t0 + (j - 2) * 2 * seg, 2 * seg)
                pltpu.make_async_copy(out_v.at[rows], out_hbm.at[rows], sem_out.at[0]).start()
        return mem

    mem0 = mem_v[...].astype(F32)
    lax.fori_loop(0, S // (4 * seg), four_segments, [mem0[:, n * LANES:(n + 1) * LANES] for n in range(NN)])
    pltpu.make_async_copy(out_v, out_hbm, sem_out.at[0]).wait()


@functools.partial(jax.jit, static_argnames=("A_seg_len",))
def pallas_recurrent_scan__memory_aug_recurrent_mem_tr__mixer_gmlp__prompt_kernel(
    A_x, A_mem0, A_Wq, A_Wk, A_Wv, A_Wo, A_seg_len, B_x, B_w_in, B_w_sp, B_b_sp, B_w_out,
):
    del B_x
    B, S, D = A_x.shape
    M = A_mem0.shape[1]
    H, DH = A_Wq.shape[1], A_Wq.shape[2]
    FH = B_w_out.shape[0]
    seg = int(A_seg_len)
    assert B == 1 and DH == LANES
    ntb = S // LANES
    scheme5, sum_groups = _parse_scheme(_SCHEME_5)
    n5, n4, n2 = len(scheme5), len(_parse_scheme(_SCHEME_4)[0]), len(_parse_scheme(_SCHEME_2)[0])
    n_sums = sum(len(g) for g in sum_groups)
    n_five = H // (D // LANES)
    x_cols = n2 * ((D // LANES - 1) // 2 * LANES) + 2 * LANES
    ky = FH // 2 // LANES * LANES
    vmem, dma = pltpu.VMEM, pltpu.SemaphoreType.DMA
    scratch = [
        vmem((S, D), BF16),
        *[vmem((2, 2 * LANES, LANES), F32)] * 2,
        vmem((S // 2, D), U32),
        *[vmem((LANES // 2, x_cols), U32)] * 2,
        vmem((M, D), BF16),
        vmem((FH, D), U32),
        vmem((FH // 2, x_cols), U32),
        vmem((S // 2, S), U32),
        vmem((FH, D), BF16),
        vmem((D // 2, FH), U32),
        vmem((D // 4, n2 * ky), U32),
        vmem((ntb, LANES), BF16),
        vmem((ntb, LANES), F32),
        *[vmem((ntb, FH, LANES), F32)] * 2,
        vmem((ntb // 4, n4, FH // 4, LANES), U32),
        vmem((n4, LANES // 2, S // 4), U32),
        *[vmem((ky // 2, (n2 + 2) * LANES), U32)] * 2,
        vmem((S, D), F32),
        vmem((3 * H + 6, D // 2, DH), U32),
        vmem((H * DH // 2, D), U32),
        vmem((3 * n_five, n_sums, DH // 2, LANES), U32),
        vmem((n_sums, n_five * DH // 2, LANES), U32),
        vmem((n5, seg // 2, LANES), U32),
        vmem((n5, seg // 2, n_five * DH), U32),
        vmem((3 * H, seg - M, DH), F32),
        vmem((H, seg - M, DH), F32),
        vmem((seg // 2, H * DH), U32),
        vmem((H, 2 * seg, DH), F32),
        vmem((S, D), A_x.dtype),
        pltpu.SMEM((8,), jnp.int32),
        dma((ntb // 4 + 1,)), dma((len(IN_ARRIVAL) + 1,)), dma((1,)),
        dma((ntb // 4,)), dma((ntb // 4,)), dma((ntb // 4,)), dma((1,)),
    ]
    hbm = pl.BlockSpec(memory_space=pltpu.HBM)
    out = pl.pallas_call(
        functools.partial(_kernel, seg=seg),
        out_shape=jax.ShapeDtypeStruct((S, D), A_x.dtype),
        in_specs=[hbm] * 10,
        out_specs=hbm,
        scratch_shapes=scratch,
        compiler_params=pltpu.CompilerParams(vmem_limit_bytes=124 * 2**20),
    )(
        A_x.reshape(S, D),
        A_mem0.reshape(M, D),
        A_Wq.reshape(D // 2, 2, H, DH),
        A_Wk.reshape(D // 2, 2, H, DH),
        A_Wv.reshape(D // 2, 2, H, DH),
        A_Wo.reshape(H * DH, D),
        B_w_in.T,
        B_w_sp,
        B_b_sp.reshape(ntb, LANES),
        B_w_out,
    )
    return out.reshape(B, S, D)
```

```python
import functools
import math

import jax
import jax.numpy as jnp
from jax import lax
import jax.experimental.pallas as pl
import jax.experimental.pallas.tpu as pltpu

F32 = jnp.float32
BF16 = jnp.bfloat16
U32 = jnp.uint32
LANES = 128
LOG2E = 1.4426950408889634
EPS = 1e-5

_SCHEME_5 = """
+Q0 | +00 -20 -30 -04 -01 +10 | +S0 | 0
+R0 | +00 -02 -03 -40 +01 -10 | +U0 | 0
+Q1 | +11 -21 -31 -14 +32 | +S1 | 0
+R1 | +11 -12 -13 -41 +23 | +U1 | 0
+R2 | -22 +20 +21 +42 -10 | +V2 | 1
+P2 | +22 -02 -12 -24 +01 | +S2 | 1
+R3 | -33 +30 +31 +43 -32 +23 | +V3 | 1
+P3 | +33 -03 -13 -34 -32 +23 | +S3 | 1
+Q4 | +44 -40 -41 -24 -34 | +V4 | 1
+P4 | +44 -04 -14 -42 -43 | +U4 | 1
+Q0 +Q2 | +20 -10 | +V0 +V2 | 2
+P0 +P2 | +02 -01 | +U0 +U2 | 2
+Q0 +P2 | -02 +20 +01 -10 | +U0 -V2 | 2
+Q0 +Q3 | +30 | +V0 +V3
+P0 +P3 | +03 | +U0 +U3
+Q0 +P3 | -03 +30 | +U0 -V3 | 2
+R0 +R4 | -40 | +V0 +V4
+P0 +P4 | +04 | +S0 +S4
+R0 +P4 | -04 +40 | +S0 +V4 | 2
+R0 +R1 +R2 | -10 | +V0 +V1 +V2
+P0 +P1 +P2 | +01 | +S0 +S1 +S2
+R0 +P1 +P2 | -01 +10 | +S0 +V1 +V2 | 3
+Q1 +Q2 | +21 -10 -32 | +V1 +V2 | 3
+P1 +P2 | +12 -01 -23 | +U1 +U2 | 3
+Q1 +P2 | -12 +21 | +U1 -V2 | 3
+Q3 +Q1 +Q2 | +32 | +S3 +S1 +S2
+R3 +R1 +R2 | +23 | +U3 +U1 +U2
+R3 -Q1 -Q2 | +32 -23 | +S3 +U1 +U2 | 4
+Q1 +Q3 | +31 -32 | +V1 +V3 | 4
+P1 +P3 | +13 -23 | +U1 +U3 | 4
+Q1 +P3 | -13 +31 -32 +23 | +U1 -V3 | 4
+R1 +R4 | -41 | +V1 +V4
+P1 +P4 | +14 | +S1 +S4
+R1 +P4 | -14 +41 | +S1 +V4 | 4
+Q2 +Q4 | +24 | +S2 +S4
+R2 +R4 | +42 | +U2 +U4
+R2 -Q4 | +24 -42 | +S2 +U4 | 4
+Q3 +Q4 | +34 | +S3 +S4
+R3 +R4 | +43 | +U3 +U4
+R3 -Q4 | +34 -43 | +S3 +U4 | 4
"""
_SCHEME_4 = """
+Q0 | +00 -20 -03 -01 +10 | +S0
+R0 | +00 -02 -30 +01 -10 | +U0
+Q0 +Q2 | +20 -10 | +V0 +V2
+P0 +P2 | +02 -01 | +U0 +U2
+Q0 +P2 | -02 +20 +01 -10 | +U0 -V2
+R0 +R3 | -30 | +V0 +V3
+P0 +P3 | +03 | +S0 +S3
+R0 +P3 | -03 +30 | +S0 +V3
+R0 +R1 +R2 | -10 | +V0 +V1 +V2
+P0 +P1 +P2 | +01 | +S0 +S1 +S2
+R0 +P1 +P2 | -01 +10 | +S0 +V1 +V2
+Q1 | +11 -21 -13 | +S1
+R1 | +11 -12 -31 | +U1
+Q1 +Q2 | +21 -10 | +V1 +V2
+P1 +P2 | +12 -01 | +U1 +U2
+Q1 +P2 | -12 +21 | +U1 -V2
+R1 +R3 | -31 | +V1 +V3
+P1 +P3 | +13 | +S1 +S3
+R1 +P3 | -13 +31 | +S1 +V3
+R2 | -22 +20 +21 +32 -10 | +V2
+P2 | +22 -02 -12 -23 +01 | +S2
+Q2 +Q3 | +23 | +S2 +S3
+R2 -Q3 | +23 -32 | +S2 +U3
+R2 +R3 | +32 | +U2 +U3
+Q3 | +33 -30 -31 -23 | +V3
+P3 | +33 -03 -13 -32 | +U3
"""
_SCHEME_2 = """
+Q0 | +00 -10 | +S0
+R0 | +00 -01 | +U0
+P0 +P1 | +01 | +U0 +U1
+Q0 +P1 | -01 +10 | +U0 -V1
+Q0 +Q1 | +10 | +V0 +V1
+P1 | +11 -01 | +S1
+R1 | -11 +10 | +V1
"""

IN_ROWS = 96
IN_ARRIVAL = (2, 4, 6)
MIX_ROWS = 144
SCORE_DELAY = 240
VALUE_DELAY = 260
SOFTMAX_DELAY = 780


def _parse_scheme(text):
    sign = {"+": 1, "-": -1}
    products, groups = [], {}
    for line in text.strip().split("\n"):
        left, weight, out, *group = (part.split() for part in line.split("|"))
        left = [(sign[t[0]], t[1], int(t[2])) for t in left]
        weight = [(sign[t[0]], int(t[1]), int(t[2])) for t in weight]
        out = [(sign[t[0]], t[1], int(t[2])) for t in out]
        if len(weight) == 1:
            out = [(s * weight[0][0], b, n) for s, b, n in out]
            products.append((left, [(1,) + weight[0][1:]], out, None))
        else:
            slot = sum(len(g) for g in groups.values())
            products.append((left, sorted(weight, reverse=True), out, slot))
            groups.setdefault(str(group), []).append((products[-1][1], slot))
    return products, [groups[g] for g in sorted(groups)]


def _signed_sum(terms):
    terms = sorted(terms, key=lambda t: -t[0])
    total = terms[0][1] if terms[0][0] > 0 else -terms[0][1]
    for s, v in terms[1:]:
        total = total + v if s > 0 else total - v
    return total


def _left_terms(left):
    return [(s * t, half, k) for s, b, k in left
            for t, half in {"P": [(1, 0)], "Q": [(1, 1)], "R": [(1, 0), (-1, 1)]}[b]]


def _scatter(acc, out, m):
    for s, b, n in out:
        if (b, n) not in acc:
            acc[b, n] = m if s > 0 else -m
        else:
            acc[b, n] = acc[b, n] + m if s > 0 else acc[b, n] - m


def _fast_matmul(scheme, product, direct, emit):
    acc = {}
    blocks = max(o[2] for p in scheme for o in p[2]) + 1
    last = {(half, n): max(r for r, p in enumerate(scheme) if any(o[1:] in (("UV"[half], n), ("S", n)) for o in p[2]))
            for half in range(2) for n in range(blocks)}
    for r, (_, _, out, _) in enumerate(scheme):
        _scatter(acc, out, product(r))
        for (half, n), when in last.items():
            if when == r:
                total = acc["UV"[half], n] + acc["S", n]
                emit(half, n, total if direct is None else total + direct(half, n))


def _dot(a, b):
    return jnp.dot(a, b, preferred_element_type=F32)


def _dot_nt(a, b):
    return lax.dot_general(a, b, (((1,), (1,)), ((), ())), preferred_element_type=F32)


def _stack(parts):
    return jnp.concatenate(parts, axis=0)


def _rows(i, n):
    if isinstance(i, int):
        return pl.ds(i * n, n)
    return pl.ds(pl.multiple_of(i * n, n), n)


def _words(x):
    return pltpu.bitcast(x.astype(BF16), U32)


def _zip_rows(x):
    return _stack([pltpu.pack_elementwise([x[r:r + 8], x[r + 8:r + 16]], packed_dtype=BF16)
                   for r in range(0, x.shape[0], 16)])


def _word_sum(terms):
    if len(terms) == 1 and terms[0][0] > 0:
        return terms[0][1]
    return pltpu.pack_elementwise(
        [_signed_sum([(s, pltpu.unpack_elementwise(w, index=e, packed_dtype=BF16, unpacked_dtype=F32))
                      for s, w in terms]) for e in range(2)], packed_dtype=BF16)


class _Packed:
    def __init__(self, words):
        self.words = words

    def __getitem__(self, idx):
        idx = idx if isinstance(idx, tuple) else (idx,)
        at = len(self.words.shape) - 2
        if len(idx) > at and not isinstance(idx[at], slice):
            start = idx[at].start // 2
            if not isinstance(start, int):
                start = pl.multiple_of(start, 8)
            idx = idx[:at] + (pl.ds(start, idx[at].size // 2),) + idx[at + 1:]
        return pltpu.bitcast(self.words[idx], BF16)


def _spread(jobs, n):
    slots = [[] for _ in range(n)]
    total, spent = max(1, sum(cost for cost, _ in jobs)), 0
    for cost, job in jobs:
        slots[spent * n // total].append(job)
        spent += cost
    return slots


def _at_once(jobs):
    for _, job in jobs:
        job(lambda v: v)


class _Stream:
    def __init__(self):
        self.now = 0
        self.waiting = []

    def defer(self, ready, cost, fn):
        self.waiting.append((ready, cost, fn))
        self.waiting.sort(key=lambda w: w[0])

    def _emit_next(self):
        ready, cost, fn = self.waiting.pop(0)
        self.now = max(self.now, ready) + cost
        fn()

    def run(self, cost, fn):
        while self.waiting and self.waiting[0][0] <= self.now:
            self._emit_next()
        self.now += cost
        return fn()

    def until(self, done):
        while not done():
            self._emit_next()


def _kernel(
    x_hbm, mem_hbm, wq_hbm, wk_hbm, wv_hbm, wo_hbm, wint_hbm, wsp_hbm, b_hbm, wout_hbm,
    out_hbm,
    x_v, lna_v, lnb_v, xn_w, xa_w, xb_w, mem_v, wint_w, win_w, wsp_w, wout_v, woutt_w, wol_w, b_v, bias_v,
    z1_v, d_v, z2_w, ws_w, ya_w, yb_w, gate_v, wqkv_w, wo_w, wfq_w, wfo_w,
    lq_w, lo_w, qkv_carry, o_carry, o16_w, o32_v, out_v, zero,
    sem_x, sem_in, sem_small, sem_sp, sem_qkv, sem_wo, sem_out,
    *, seg,
):
    S, D = out_v.shape
    M = mem_v.shape[0]
    H = o_carry.shape[0]
    DH = LANES
    FH = wout_v.shape[0]
    HF = FH // 2
    NTB = S // LANES
    NQ = NTB // 4
    NN = D // LANES
    assert (M, seg, NN, H, NQ) == (8, 32, 5, 32, 4)
    scheme5, sum_groups = _parse_scheme(_SCHEME_5)
    scheme4, _ = _parse_scheme(_SCHEME_4)
    scheme2, _ = _parse_scheme(_SCHEME_2)
    n2 = len(scheme2)
    n_five = H // NN
    xn, xa, xb, win, woutt, wol, z2, ws, ya, yb, wo, wfq, wfo, lq, lo, o16 = map(_Packed, (
        xn_w, xa_w, xb_w, win_w, woutt_w, wol_w, z2_w, ws_w, ya_w, yb_w, wo_w, wfq_w, wfo_w, lq_w, lo_w, o16_w))

    def x_copy(i):
        r0, r1 = (2 * i, 2 * i + 2) if i < 2 else (4 * i - 4, 4 * i)
        rows = pl.ds(r0 * LANES, (r1 - r0) * LANES)
        return pltpu.make_async_copy(x_hbm.at[rows], x_v.at[rows], sem_x.at[i])

    cuts = [0] + [c * IN_ROWS for c in IN_ARRIVAL] + [FH]

    def win_copies(c):
        rows = [pl.ds((half * FH + cuts[c]) // 2, (cuts[c + 1] - cuts[c]) // 2) for half in range(2)]
        return [pltpu.make_async_copy(wint_hbm.bitcast(U32).at[r], wint_w.at[r], sem_in.at[c]) for r in rows]

    def wsp_copy(i):
        rows = _rows(i, 2 * LANES)
        return pltpu.make_async_copy(wsp_hbm.bitcast(U32).at[rows], wsp_w.at[rows], sem_sp.at[i])

    chunks = [range(NN * i, min(NN * (i + 1), H // 2)) for i in range(NQ)]

    def wo_copy(i):
        rows = pl.ds(chunks[i][0] * DH, len(chunks[i]) * DH)
        return pltpu.make_async_copy(wo_hbm.bitcast(U32).at[rows], wo_w.at[rows], sem_wo.at[i])

    def start_attention_weights(i):
        wo_copy(i).start()
        for j in chunks[i]:
            for m, w in enumerate((wk_hbm, wq_hbm, wv_hbm)):
                for b in range(2):
                    pltpu.make_async_copy(
                        w.bitcast(U32).at[:, b, j, :], wqkv_w.at[6 * j + 3 * b + m], sem_qkv.at[i]).start()

    def wait_attention_weights(i):
        wo_copy(i).wait()
        filled = wqkv_w.at[pl.ds(6 * chunks[i][0], 6 * len(chunks[i]))]
        pltpu.make_async_copy(filled, filled, sem_qkv.at[i]).wait()

    small_copies = [pltpu.make_async_copy(src, dst, sem_small.at[0])
                    for src, dst in ((wout_hbm, wout_v), (b_hbm, b_v), (mem_hbm, mem_v))]

    for e in range(zero.shape[0]):
        zero[e] = 0
    x_copy(0).start()
    for c in range(len(cuts) - 1):
        for cp in win_copies(c):
            cp.start()
    x_copy(1).start()

    def timed_after(result):
        always = jnp.full((8, LANES), zero[zero.shape[0] - 1], jnp.int32) == 0

        def after(v):
            reps = (v.shape[0] // 8, v.shape[1] // LANES)
            token = pltpu.bitcast(result[:8, :LANES], v.dtype)
            return jnp.where(jnp.tile(always, reps), v, jnp.tile(token, reps))

        return after

    def run_jobs(groups, result):
        jobs = [job for group in groups for job in group]
        if jobs:
            after = timed_after(result)
            for job in jobs:
                job(after)

    KX = (NN - 1) // 2 * LANES

    def norm_jobs(p, dst_w, ln_v):
        def rows(r, e):
            start = p * (2 * LANES) + pl.multiple_of(zero[e], 64) + r
            return x_v[pl.ds(start, 16), :].astype(F32)

        def mean(r, after):
            ln_v[0, pl.ds(r, 16), :] = after(jnp.broadcast_to(
                jnp.mean(rows(r, 0), axis=-1, keepdims=True), (16, LANES)))

        def centred(r, e):
            return rows(r, e) - jnp.tile(ln_v[0, pl.ds(r, 16), :], (1, NN))

        def scale(r, after):
            d = centred(r, 1)
            ln_v[1, pl.ds(r, 16), :] = after(jnp.broadcast_to(
                lax.rsqrt(jnp.mean(d * d, axis=-1, keepdims=True) + EPS), (16, LANES)))

        def apply(r, after):
            xn_w[pl.ds(p * LANES + r // 2, 8), :] = after(
                _words(centred(r, 2) * jnp.tile(ln_v[1, pl.ds(r, 16), :], (1, NN))))

        def operands(r, after):
            start = p * LANES + pl.multiple_of(zero[3], 64)
            w = [xn_w[pl.ds(start + (n * LANES + r) // 2, 8), :] for n in range(2)]
            for n in range(2):
                dst_w[pl.ds(r // 2, 8), pl.ds(n2 * KX + n * LANES, LANES)] = after(w[n][:, 2 * KX:])
            for e, (_, weight, _, _) in enumerate(scheme2):
                dst_w[pl.ds(r // 2, 8), pl.ds(e * KX, KX)] = after(_word_sum(
                    [(s, w[n][:, k * KX:(k + 1) * KX]) for s, k, n in weight]))

        both = range(0, 2 * LANES, 16)
        return ([(2, functools.partial(mean, r)) for r in both] + [(3, functools.partial(scale, r)) for r in both]
                + [(4, functools.partial(apply, r)) for r in both]
                + [(6, functools.partial(operands, r)) for r in range(0, LANES, 16)])

    def fold(z):
        return jnp.sum(z.reshape(z.shape[0] // 8, 8, LANES), axis=0)

    def in_proj(p, src, early=(), late=(), steady=(), before=lambda c: None, hold=0):
        n_chunks = FH // IN_ROWS
        per = n2 * (KX // LANES) + 4
        slots = iter(zip(*[[[]] * a + _spread(jobs, n_chunks * per - a - b) + [[]] * b
                           for jobs, a, b in ((early, hold * per, 10), (late, 40, 0), (steady, 0, 0))]))
        shift, s1, s2 = {}, {}, {}
        for c in range(n_chunks):
            rows = pl.ds(c * IN_ROWS, IN_ROWS)
            before(c)

            def tile(lhs, rhs):
                part = _dot_nt(win[rows, pl.ds(lhs, LANES)], src[:, pl.ds(rhs, LANES)])
                run_jobs(next(slots), part)
                return part

            def product(r):
                return _signed_sum([(1, tile(r * KX + k, r * KX + k)) for k in range(0, KX, LANES)])

            def direct(half, n):
                return tile(n2 * KX + half * LANES, n2 * KX + n * LANES)

            def emit(half, n, z):
                c0 = math.sqrt(2.0 / math.pi)
                z = z * (1.0 + jnp.tanh(z * (c0 + (c0 * 0.044715) * (z * z))))
                if half == 0:
                    z1_v[2 * p + n, rows, :] = z
                    return
                if c == 0:
                    shift[n] = z[:8]
                d = z - jnp.tile(shift[n], (IN_ROWS // 8, 1))
                d_v[2 * p + n, rows, :] = d
                s1[n] = fold(d) if c == 0 else s1[n] + fold(d)
                s2[n] = fold(d * d) if c == 0 else s2[n] + fold(d * d)

            _fast_matmul(scheme2, product, direct, emit)
        stats = []
        for n in range(2):
            off = jnp.sum(s1[n] + (FH // 8) * shift[n], axis=0, keepdims=True) * (1.0 / FH) - shift[n]
            var = jnp.sum(s2[n] - off * (2.0 * s1[n] - (FH // 8) * off), axis=0, keepdims=True) * (1.0 / FH)
            stats.append((off, 0.25 * lax.rsqrt(jnp.maximum(var, 0.0) + 4.0 * EPS)))
        return stats

    def rescale_jobs(q, stats, timed_input=False):
        def job(r, after):
            off = [jnp.tile(after(stats[n][0]) if timed_input else stats[n][0], (2, 1)) for n in range(4)]
            base = {}
            for k in range(4):
                for half in range(2):
                    base["PQ"[half], k] = (d_v[4 * q + k, pl.ds(half * HF + r, 16), :] - off[k]) * stats[k][1]
                base["R", k] = base["P", k] - base["Q", k]
            for e, (left, _, _, _) in enumerate(scheme4):
                w = _zip_rows(_signed_sum([(s, base[b, k]) for s, b, k in left]))
                z2_w[q, e, pl.ds(r // 2, 8), :] = w if timed_input else after(w)
            return w

        return [(1, functools.partial(job, r)) for r in range(0, HF, 16)]

    def weights_arrived(c):
        for cp in win_copies(c):
            cp.wait()
        if c == len(cuts) - 3:
            for i in range(2, NQ + 1):
                x_copy(i).start()
            for cp in small_copies:
                cp.start()
        if c == len(cuts) - 2:
            wsp_copy(0).start()
            wsp_copy(1).start()
            start_attention_weights(0)
            start_attention_weights(1)
        for r in range(cuts[c], cuts[c + 1], 16):
            w = [wint_w[pl.ds((half * FH + r) // 2, 8), :] for half in range(2)]
            w[0] = _zip_rows(pltpu.bitcast(w[0], BF16).astype(F32))
            for e, (left, _, _, _) in enumerate(scheme2):
                win_w[pl.ds(r // 2, 8), pl.ds(e * KX, KX)] = _word_sum(
                    [(s, w[half][:, k * KX:(k + 1) * KX]) for s, half, k in _left_terms(left)])
            for half in range(2):
                win_w[pl.ds(r // 2, 8), pl.ds(n2 * KX + half * LANES, LANES)] = w[half][:, 2 * KX:]

    KY = HF // LANES * LANES
    DC = LANES // 2
    d_chunks = [(d, 2 * LANES + d) for d in range(0, 2 * LANES, DC)] + [(4 * LANES, 4 * LANES + DC)]

    def out_weight_jobs():
        def hidden_order(r, n, d):
            w = wout_v[pl.ds(r, n), pl.ds(d, LANES)]
            for _ in range(2):
                w = pltpu.bitcast(_zip_rows(w.astype(F32)), BF16)
            return w

        def transpose(col, d, after):
            if col < 2 * KY:
                w = hidden_order(col // KY * HF + col % KY, LANES, d)
            else:
                w = _stack([hidden_order(k * HF + KY, HF - KY, d) for k in range(2)])
            w = pltpu.bitcast(after(pltpu.bitcast(w, U32)), BF16)
            woutt_w[pl.ds(d // 2, LANES // 2), pl.ds(col, w.shape[0])] = pltpu.bitcast(w.T, U32)

        def operands(c, r, after):
            w = [woutt_w[pl.ds((d + r) // 2, 8), pl.ds(0, 2 * KY)] for d in d_chunks[c]]
            for e, (left, _, _, _) in enumerate(scheme2):
                wol_w[pl.ds((c * DC + r) // 2, 8), pl.ds(e * KY, KY)] = after(_word_sum(
                    [(s, w[half][:, k * KY:(k + 1) * KY]) for s, half, k in _left_terms(left)]))

        return ([(2, functools.partial(transpose, col, d)) for d in range(0, D, LANES) for col in range(0, FH, LANES)]
                + [(4, functools.partial(operands, c, r)) for c in range(len(d_chunks)) for r in range(0, DC, 16)])

    def stage_jobs(o):
        def job(r, q, after):
            w = {(k, n): wsp_w[pl.ds(o * (2 * LANES) + (n * LANES + r) // 2, 8), pl.ds((4 * q + k) * LANES, LANES)]
                 for k in range(4) for n in range(4)}
            for e, (_, weight, _, _) in enumerate(scheme4):
                ws_w[e, pl.ds(r // 2, 8), pl.ds(q * LANES, LANES)] = after(_word_sum(
                    [(s, w[k, n]) for s, k, n in weight]))

        return [(1, functools.partial(job, r, q)) for q in range(NQ) for r in range(0, LANES, 16)]

    x_copy(0).wait()
    for r in range(0, 2 * LANES, 16):
        x = x_v[pl.ds(r, 16), :].astype(F32)
        d = x - jnp.mean(x, axis=-1, keepdims=True)
        xn_w[pl.ds(r // 2, 8), :] = _words(d * lax.rsqrt(jnp.mean(d * d, axis=-1, keepdims=True) + EPS))
    _at_once(norm_jobs(0, xa_w, lna_v)[-LANES // 16:])

    def before(c):
        if c * IN_ROWS in cuts:
            weights_arrived(cuts.index(c * IN_ROWS))
        if c == IN_ARRIVAL[-1]:
            x_copy(1).wait()

    stats = in_proj(0, xa, early=norm_jobs(1, xb_w, lna_v), before=before, hold=IN_ARRIVAL[-1])

    def phase1(o, stats):
        for k in range(NQ - 1):
            @pl.when(o == k)
            def _():
                x_copy(k + 2).wait()

        ahead = norm_jobs(2 * o + 3, xb_w, lnb_v)
        odd = in_proj(2 * o + 1, xb, early=norm_jobs(2 * o + 2, xa_w, lna_v), steady=ahead[:32])
        return in_proj(2 * o + 2, xa, late=rescale_jobs(o, stats + odd), steady=ahead[32:])

    stats = lax.fori_loop(0, NQ - 1, phase1, stats)
    for cp in small_copies + [wsp_copy(0)]:
        cp.wait()
    for i in range(2, NQ):
        wsp_copy(i).start()
    start_attention_weights(2)
    stats = stats + in_proj(NTB // 2 - 1, xb, early=out_weight_jobs(), steady=stage_jobs(0))
    results = []
    for _, job in rescale_jobs(NQ - 1, stats, timed_input=True):
        results.append(job(timed_after(results[-2]) if len(results) >= 2 else (lambda v: v)))
    bias_v[...] = 0.25 * b_v[...].astype(F32)

    def repack_jobs(j):
        def job(m, r, after):
            t, rows = 6 * j + m, pl.ds(r, 8)
            a = wqkv_w[t, rows, :]
            b = wqkv_w[t + 3, rows, :]
            wqkv_w[t, rows, :] = after((a & U32(0xFFFF)) | (b << 16))
            wqkv_w[t + 3, rows, :] = after((a >> 16) | (b & U32(0xFFFF0000)))

        return [(16, functools.partial(job, m, r)) for m in range(3) for r in range(0, D // 2, 8)]

    def weight_sum_jobs(load, store, r):
        def job(e, members, after):
            words = {}
            for weight, slot in members:
                for _, k, n in weight:
                    if (k, n) not in words:
                        words[k, n] = load(k, n, pl.multiple_of(r + zero[e], 8))
                store(slot, pl.multiple_of(r, 8), after(_word_sum([(s, words[k, n]) for s, k, n in weight])))

        return [(sum(3 * len(weight) for weight, _ in members), functools.partial(job, e, members))
                for e, members in enumerate(sum_groups)]

    def qkv_sum_jobs(g, m, row):
        def load(k, n, r):
            return wqkv_w[3 * (NN * g + n) + m, pl.ds(r + k * (DH // 2), 8), :]

        def store(slot, r, w):
            wfq_w[3 * g + m, slot, pl.ds(r, 8), :] = w

        return weight_sum_jobs(load, store, row)

    def out_sum_jobs(g, row):
        def load(k, n, r):
            return wo_w[pl.ds(g * (NN * DH // 2) + r + k * (DH // 2), 8), pl.ds(n * LANES, LANES)]

        def store(slot, r, w):
            wfo_w[slot, pl.ds(g * (DH // 2) + r, 8), :] = w

        return weight_sum_jobs(load, store, row)

    def mix(o, jobs):
        rc = MIX_ROWS
        slots = iter(_spread(jobs, HF // rc * len(scheme4) * NQ))
        for c in range(HF // rc):
            ys = {}

            def product(r):
                total = None
                for q in range(NQ):
                    part = _dot_nt(z2[q, r, pl.ds(c * rc, rc), :], ws[r, :, pl.ds(q * LANES, LANES)])
                    total = part if q == 0 else total + part
                    run_jobs([next(slots)], part)
                return total

            def emit(half, n, g):
                ys[half, n] = z1_v[4 * o + n, pl.ds(half * HF + c * rc, rc), :] * (g + bias_v[pl.ds(4 * o + n, 1), :])
                u = n // 2
                if not all((k, 2 * u + t) in ys for k in range(2) for t in range(2)):
                    return
                y_w = (ya_w, yb_w)[u]
                m = max(0, min(rc, KY - c * rc))
                if m:
                    for e, (_, weight, _, _) in enumerate(scheme2):
                        y_w[pl.ds(c * rc // 2, m // 2), pl.ds(e * LANES, LANES)] = _zip_rows(_signed_sum(
                            [(s, ys[k, 2 * u + t][:m]) for s, k, t in weight]))
                if m < rc:
                    for k in range(2):
                        for t in range(2):
                            y_w[pl.ds((k * (HF - KY) + c * rc + m - KY) // 2, (rc - m) // 2),
                                pl.ds((n2 + t) * LANES, LANES)] = _zip_rows(ys[k, 2 * u + t][m:])

            _fast_matmul(scheme4, product, None, emit)

    def out_proj(p, y, jobs):
        slots = iter(_spread(jobs, len(d_chunks) * n2))
        tiles = {}
        for c, d0 in enumerate(d_chunks):
            def part(r, k0, k1):
                total = _dot(wol[pl.ds(c * DC, DC), pl.ds(r * KY + k0, k1 - k0)],
                             y[pl.ds(k0, k1 - k0), pl.ds(r * LANES, LANES)])
                if k1 == KY:
                    run_jobs([next(slots)], total)
                return total

            early = [part(r, 0, KY - LANES) for r in range(3)] if c == 0 else []

            def product(r):
                return early[r] + part(r, KY - LANES, KY) if r < len(early) else part(r, 0, KY)

            def direct(half, n):
                return _dot(woutt[pl.ds(d0[half], DC), pl.ds(2 * KY, FH - 2 * KY)],
                            y[pl.ds(0, FH - 2 * KY), pl.ds((n2 + n) * LANES, LANES)])

            def emit(half, n, h):
                d = d0[half] // LANES * LANES
                done = tiles.setdefault((d, n), {})
                done[d0[half]] = h + h * jnp.tanh(h)
                if len(done) * DC == LANES:
                    gate_v[_rows(2 * p + n, LANES), pl.ds(d, LANES)] = _stack([done[k] for k in sorted(done)]).T

            _fast_matmul(scheme2, product, direct, emit)

    def phase2(o, _):
        for k in range(NQ):
            @pl.when(o == k)
            def _():
                if k + 1 < NQ:
                    wsp_copy(k + 1).wait()
                wait_attention_weights(k)
                if k == 1:
                    start_attention_weights(3)

        whole, shared, row = (3 * o + 1) // 2, o // 2 * 3 + 1, o % 2 * (DH // 4)
        first = [job for r in range(0, DH // 2, 8) for job in out_sum_jobs(whole, r)]
        repack = [job for u in range(NN) for job in repack_jobs(jnp.minimum(o * NN + u, H // 2) if u else o * NN)]
        jobs = [job for a, b in zip(first, _spread([(1, job) for job in repack], len(first))) for job in [a] + b]
        for m in range(3):
            for r in range(0, DH // 2, 8):
                jobs += qkv_sum_jobs(whole, m, r)
            for r in range(0, DH // 4, 8):
                jobs += qkv_sum_jobs(shared, m, row + r)
        for r in range(0, DH // 4, 8):
            jobs += out_sum_jobs(shared, row + r)
        mix(o, jobs)
        ahead = _spread([(1, job) for job in stage_jobs(jnp.minimum(o + 1, NQ - 1))], 2)
        out_proj(2 * o, ya, ahead[0])
        out_proj(2 * o + 1, yb, ahead[1])

    lax.fori_loop(0, NQ, phase2, None)

    L = M + seg
    T = seg - M
    row = lax.broadcasted_iota(jnp.int32, (L, L), 0)
    col = lax.broadcasted_iota(jnp.int32, (L, L), 1)
    keep = (row < M) | (row >= col)
    heads = list(range(NN * n_five, H)) + list(range(NN * n_five))
    order = [3 * (hd + b) + m for hd in heads[::2] for m in range(3) for b in range(2)]
    last_use = [max(r for r, p in enumerate(scheme5) if any(o[2] == n for o in p[2])) for n in range(NN)]

    def left_sum_jobs(block, store):
        base = {}

        def term(b, k):
            if (b, k) not in base:
                base[b, k] = term("P", k) - term("Q", k) if b == "R" else block("PQ".index(b), k)
            return base[b, k]

        def job(r, left, after):
            store(r, after(_words(_signed_sum([(s, term(b, k)) for s, b, k in left]))))

        return [(1, functools.partial(job, r, left)) for r, (left, _, _, _) in enumerate(scheme5)]

    def gather(acc, n):
        return _stack([acc["U", n] + acc["S", n], acc["V", n] + acc["S", n]])

    def four_segments(grp, mem):
        t0 = pl.multiple_of(grp * 4 * seg, 4 * seg)
        mxu = _Stream()

        def tokens(r, n, k):
            return xn[pl.ds(t0 + r, n), pl.ds(k * LANES, LANES)].astype(F32)

        def finish(r, n, k, s):
            rows, cols = pl.ds(t0 + r, n), pl.ds(k * LANES, LANES)
            out_v[rows, cols] = (x_v[rows, cols].astype(F32) + s * gate_v[rows, cols]).astype(out_v.dtype)

        for j in range(4):
            tiles = {}
            done = {}

            def attend(hd, j=j, tiles=tiles, done=done):
                st = {}

                def scores():
                    sc = _dot_nt(tiles.pop(3 * hd + 1), tiles.pop(3 * hd).astype(BF16))
                    sc = jnp.where(keep, sc * (DH ** -0.5 * LOG2E), -1e9 * LOG2E)
                    p = jnp.exp2(sc - jnp.max(sc, axis=1, keepdims=True))
                    st["p"] = p * pl.reciprocal(jnp.sum(p, axis=1, keepdims=True), approx=False, full_range=False)
                    st["t"] = mxu.now + SOFTMAX_DELAY
                    values_ready()

                def values_ready():
                    if "p" in st and 3 * hd + 2 in tiles:
                        mxu.defer(max(st["t"], done["v", hd] + VALUE_DELAY), L // 4, values)

                def values():
                    o = _dot(st.pop("p"), tiles.pop(3 * hd + 2).astype(BF16))
                    parts = [o[:M]] + ([o_carry[hd, pl.ds(0, M * j), :]] if j else [])
                    if j < 3:
                        new = T - M * j
                        o16_w[:, pl.ds(hd * DH, DH)] = _words(_stack(parts + [o[M:M + new]]))
                        o_carry[hd, pl.ds(0, seg - new), :] = o[M + new:]
                    else:
                        o32_v[hd] = _stack(parts + [o[M:]])
                    done["o", hd] = mxu.now
                    g = hd // NN
                    if j == 3 and g < n_five and all(("o", NN * g + k) in done for k in range(NN)):
                        def keep_left(r, a):
                            lo_w[r, :, pl.ds(g * DH, DH)] = a

                        _at_once(left_sum_jobs(lambda t, k: o32_v[NN * g + k, pl.ds(t * seg, seg), :], keep_left))

                def on_tile(m):
                    if m == 1:
                        mxu.defer(mxu.now + SCORE_DELAY, L // 4, scores)
                    elif m == 2:
                        done["v", hd] = mxu.now
                        values_ready()

                return on_tile

            notify = [attend(hd) for hd in range(H)]

            def tile_done(t, y, j=j, tiles=tiles, notify=notify):
                old = 0 if j == 0 else T - M * (j - 1)
                parts = [y[:M]] + ([qkv_carry[t, pl.ds(0, old), :]] if old else [])
                tiles[t] = _stack(parts + [y[M:M + seg - old]])
                if j < 3:
                    qkv_carry[t, pl.ds(0, T - M * j), :] = y[M + seg - old:]
                notify[t // 3](t % 3)

            def need(hds, done=done):
                mxu.until(lambda: all(("o", hd) in done for hd in hds))

            if j == 0:
                h = [_stack([mem[k], tokens(0, 2 * seg, k)[:seg + T]]) for k in range(NN)]
                hh = jnp.concatenate(h, axis=1).astype(BF16)

                def keep_left(r, a):
                    lq_w[r] = a

                plain = order[:3 * (H - NN * n_five)]
                slots = iter(_spread(left_sum_jobs(lambda t, k: h[k][t * seg:(t + 1) * seg], keep_left),
                                     len(plain) * NN - 2) + [[]] * 2)
                for t in plain:
                    for k in range(NN):
                        part = mxu.run(seg // 2, lambda: _dot(
                            hh[:, k * LANES:(k + 1) * LANES],
                            pltpu.bitcast(wqkv_w[t, _rows(k, DH // 2), :], BF16)))
                        y = part if k == 0 else y + part
                        run_jobs([next(slots)], part)
                    tile_done(t, y)
                for g in range(n_five):
                    for m in range(3):
                        first = 3 * NN * g + m
                        acc = {}
                        for r, (_, weight, out, slot) in enumerate(scheme5):
                            def product():
                                if slot is None:
                                    _, k, n = weight[0]
                                    w = pltpu.bitcast(wqkv_w[first + 3 * n, _rows(k, DH // 2), :], BF16)
                                else:
                                    w = wfq[3 * g + m, slot]
                                return _dot(lq[r], w)

                            _scatter(acc, out, mxu.run(seg // 4, product))
                            for n in range(NN):
                                if last_use[n] == r:
                                    tile_done(first + 3 * n, gather(acc, n))
            else:
                r0 = seg + T * j
                a0 = r0 // 16 * 16
                h = [_stack([mem[k], tokens(a0, seg, k)[r0 - a0:r0 - a0 + T]]).astype(BF16) for k in range(NN)]
                partial = {}
                for k in range(NN):
                    for t in order[:4]:
                        y = mxu.run(seg // 4, lambda: _dot(
                            h[k], pltpu.bitcast(wqkv_w[t, _rows(k, DH // 2), :], BF16)))
                        partial[t] = y if k == 0 else partial[t] + y
                        if k == NN - 1:
                            tile_done(t, partial.pop(t))
                hh = jnp.concatenate(h, axis=1)
                for t in order[4:]:
                    tile_done(t, mxu.run(NN * seg // 4, lambda: _dot(hh, pltpu.bitcast(wqkv_w[t], BF16))))

            if j < 3:
                total = [None] * NN

                def project(hd, n):
                    need([hd])
                    y = mxu.run(seg // 4, lambda: _dot(
                        o16[:, pl.ds(hd * DH, DH)], wo[pl.ds(hd * DH, DH), pl.ds(n * LANES, LANES)]))
                    total[n] = y if total[n] is None else total[n] + y

                for hd in heads[:-8]:
                    for n in range(NN):
                        project(hd, n)
                for n in range(NN):
                    for hd in heads[-8:]:
                        project(hd, n)
                    finish(T * j, T, n, total[n][M:])
                mem = [a[:M] for a in total]
            else:
                acc = {}
                mem = [None] * NN
                rest = range(NN * n_five, H)
                need(rest)
                o_rest = jnp.concatenate([o32_v[hd] for hd in rest], axis=1).astype(BF16)
                for n in range(NN):
                    y = mxu.run(len(rest) * seg // 2, lambda: _dot(
                        o_rest, wo[pl.ds(rest[0] * DH, len(rest) * DH), pl.ds(n * LANES, LANES)]))
                    _scatter(acc, [(1, "U", n)], y[:seg])
                    _scatter(acc, [(1, "V", n)], y[seg:])
                for g0, g1 in ((0, n_five // 2), (n_five // 2, n_five)):
                    need(range(NN * g0, NN * g1))
                    span = pl.ds(g0 * DH, (g1 - g0) * DH)
                    for r, (_, weight, out, slot) in enumerate(scheme5):
                        def product():
                            if slot is None:
                                _, k, n = weight[0]
                                w = _stack([wo[pl.ds((NN * g + k) * DH, DH), pl.ds(n * LANES, LANES)]
                                            for g in range(g0, g1)])
                            else:
                                w = wfo[slot, span, :]
                            return _dot(lo[r, :, span], w)

                        _scatter(acc, out, mxu.run((g1 - g0) * seg // 4, product))
                        for n in range(NN):
                            if g1 == n_five and last_use[n] == r:
                                y = gather(acc, n)
                                finish(3 * T, seg + T, n, y[M:])
                                mem[n] = y[:M]
            assert not tiles and not mxu.waiting
            if j >= 2:
                rows = pl.ds(t0 + (j - 2) * 2 * seg, 2 * seg)
                pltpu.make_async_copy(out_v.at[rows], out_hbm.at[rows], sem_out.at[0]).start()
        return mem

    mem0 = mem_v[...].astype(F32)
    lax.fori_loop(0, S // (4 * seg), four_segments, [mem0[:, n * LANES:(n + 1) * LANES] for n in range(NN)])
    pltpu.make_async_copy(out_v, out_hbm, sem_out.at[0]).wait()


@functools.partial(jax.jit, static_argnames=("A_seg_len",))
def pallas_recurrent_scan__memory_aug_recurrent_mem_tr__mixer_gmlp__prompt_kernel(
    A_x, A_mem0, A_Wq, A_Wk, A_Wv, A_Wo, A_seg_len, B_x, B_w_in, B_w_sp, B_b_sp, B_w_out,
):
    del B_x
    B, S, D = A_x.shape
    M = A_mem0.shape[1]
    H, DH = A_Wq.shape[1], A_Wq.shape[2]
    FH = B_w_out.shape[0]
    seg = int(A_seg_len)
    assert B == 1 and DH == LANES
    ntb = S // LANES
    scheme5, sum_groups = _parse_scheme(_SCHEME_5)
    n5, n4, n2 = len(scheme5), len(_parse_scheme(_SCHEME_4)[0]), len(_parse_scheme(_SCHEME_2)[0])
    n_sums = sum(len(g) for g in sum_groups)
    n_five = H // (D // LANES)
    x_cols = n2 * ((D // LANES - 1) // 2 * LANES) + 2 * LANES
    ky = FH // 2 // LANES * LANES
    vmem, dma = pltpu.VMEM, pltpu.SemaphoreType.DMA
    scratch = [
        vmem((S, D), BF16),
        *[vmem((2, 2 * LANES, LANES), F32)] * 2,
        vmem((S // 2, D), U32),
        *[vmem((LANES // 2, x_cols), U32)] * 2,
        vmem((M, D), BF16),
        vmem((FH, D), U32),
        vmem((FH // 2, x_cols), U32),
        vmem((S // 2, S), U32),
        vmem((FH, D), BF16),
        vmem((D // 2, FH), U32),
        vmem((D // 4, n2 * ky), U32),
        vmem((ntb, LANES), BF16),
        vmem((ntb, LANES), F32),
        *[vmem((ntb, FH, LANES), F32)] * 2,
        vmem((ntb // 4, n4, FH // 4, LANES), U32),
        vmem((n4, LANES // 2, S // 4), U32),
        *[vmem((ky // 2, (n2 + 2) * LANES), U32)] * 2,
        vmem((S, D), F32),
        vmem((3 * H + 6, D // 2, DH), U32),
        vmem((H * DH // 2, D), U32),
        vmem((3 * n_five, n_sums, DH // 2, LANES), U32),
        vmem((n_sums, n_five * DH // 2, LANES), U32),
        vmem((n5, seg // 2, LANES), U32),
        vmem((n5, seg // 2, n_five * DH), U32),
        vmem((3 * H, seg - M, DH), F32),
        vmem((H, seg - M, DH), F32),
        vmem((seg // 2, H * DH), U32),
        vmem((H, 2 * seg, DH), F32),
        vmem((S, D), A_x.dtype),
        pltpu.SMEM((8,), jnp.int32),
        dma((ntb // 4 + 1,)), dma((len(IN_ARRIVAL) + 1,)), dma((1,)),
        dma((ntb // 4,)), dma((ntb // 4,)), dma((ntb // 4,)), dma((1,)),
    ]
    hbm = pl.BlockSpec(memory_space=pltpu.HBM)
    out = pl.pallas_call(
        functools.partial(_kernel, seg=seg),
        out_shape=jax.ShapeDtypeStruct((S, D), A_x.dtype),
        in_specs=[hbm] * 10,
        out_specs=hbm,
        scratch_shapes=scratch,
        compiler_params=pltpu.CompilerParams(vmem_limit_bytes=124 * 2**20),
    )(
        A_x.reshape(S, D),
        A_mem0.reshape(M, D),
        A_Wq.reshape(D // 2, 2, H, DH),
        A_Wk.reshape(D // 2, 2, H, DH),
        A_Wv.reshape(D // 2, 2, H, DH),
        A_Wo.reshape(H * DH, D),
        B_w_in.T,
        B_w_sp,
        B_b_sp.reshape(ntb, LANES),
        B_w_out,
    )
    return out.reshape(B, S, D)
```

```python
import functools
import math

import jax
import jax.numpy as jnp
from jax import lax
import jax.experimental.pallas as pl
import jax.experimental.pallas.tpu as pltpu

F32 = jnp.float32
BF16 = jnp.bfloat16
U32 = jnp.uint32
LANES = 128
LOG2E = 1.4426950408889634
EPS = 1e-5

_SCHEME_5 = """
+Q0 | +00 -20 -30 -04 -01 +10 | +S0
+R0 | +00 -02 -03 -40 +01 -10 | +U0
+Q1 | +11 -21 -31 -14 +32 | +S1
+R1 | +11 -12 -13 -41 +23 | +U1
+R2 | -22 +20 +21 +42 -10 | +V2
+P2 | +22 -02 -12 -24 +01 | +S2
+R3 | -33 +30 +31 +43 -32 +23 | +V3
+P3 | +33 -03 -13 -34 -32 +23 | +S3
+Q4 | +44 -40 -41 -24 -34 | +V4
+P4 | +44 -04 -14 -42 -43 | +U4
+Q0 +Q2 | +20 -10 | +V0 +V2
+P0 +P2 | +02 -01 | +U0 +U2
+Q0 +P2 | -02 +20 +01 -10 | +U0 -V2
+Q0 +Q3 | +30 | +V0 +V3
+P0 +P3 | +03 | +U0 +U3
+Q0 +P3 | -03 +30 | +U0 -V3
+R0 +R4 | -40 | +V0 +V4
+P0 +P4 | +04 | +S0 +S4
+R0 +P4 | -04 +40 | +S0 +V4
+R0 +R1 +R2 | -10 | +V0 +V1 +V2
+P0 +P1 +P2 | +01 | +S0 +S1 +S2
+R0 +P1 +P2 | -01 +10 | +S0 +V1 +V2
+Q1 +Q2 | +21 -10 -32 | +V1 +V2
+P1 +P2 | +12 -01 -23 | +U1 +U2
+Q1 +P2 | -12 +21 | +U1 -V2
+Q3 +Q1 +Q2 | +32 | +S3 +S1 +S2
+R3 +R1 +R2 | +23 | +U3 +U1 +U2
+R3 -Q1 -Q2 | +32 -23 | +S3 +U1 +U2
+Q1 +Q3 | +31 -32 | +V1 +V3
+P1 +P3 | +13 -23 | +U1 +U3
+Q1 +P3 | -13 +31 -32 +23 | +U1 -V3
+R1 +R4 | -41 | +V1 +V4
+P1 +P4 | +14 | +S1 +S4
+R1 +P4 | -14 +41 | +S1 +V4
+Q2 +Q4 | +24 | +S2 +S4
+R2 +R4 | +42 | +U2 +U4
+R2 -Q4 | +24 -42 | +S2 +U4
+Q3 +Q4 | +34 | +S3 +S4
+R3 +R4 | +43 | +U3 +U4
+R3 -Q4 | +34 -43 | +S3 +U4
"""
_SCHEME_4 = """
+Q0 | +00 -20 -03 -01 +10 | +S0
+R0 | +00 -02 -30 +01 -10 | +U0
+Q0 +Q2 | +20 -10 | +V0 +V2
+P0 +P2 | +02 -01 | +U0 +U2
+Q0 +P2 | -02 +20 +01 -10 | +U0 -V2
+R0 +R3 | -30 | +V0 +V3
+P0 +P3 | +03 | +S0 +S3
+R0 +P3 | -03 +30 | +S0 +V3
+R0 +R1 +R2 | -10 | +V0 +V1 +V2
+P0 +P1 +P2 | +01 | +S0 +S1 +S2
+R0 +P1 +P2 | -01 +10 | +S0 +V1 +V2
+Q1 | +11 -21 -13 | +S1
+R1 | +11 -12 -31 | +U1
+Q1 +Q2 | +21 -10 | +V1 +V2
+P1 +P2 | +12 -01 | +U1 +U2
+Q1 +P2 | -12 +21 | +U1 -V2
+R1 +R3 | -31 | +V1 +V3
+P1 +P3 | +13 | +S1 +S3
+R1 +P3 | -13 +31 | +S1 +V3
+R2 | -22 +20 +21 +32 -10 | +V2
+P2 | +22 -02 -12 -23 +01 | +S2
+Q2 +Q3 | +23 | +S2 +S3
+R2 -Q3 | +23 -32 | +S2 +U3
+R2 +R3 | +32 | +U2 +U3
+Q3 | +33 -30 -31 -23 | +V3
+P3 | +33 -03 -13 -32 | +U3
"""
_SCHEME_2 = """
+Q0 | +00 -10 | +S0
+R0 | +00 -01 | +U0
+P0 +P1 | +01 | +U0 +U1
+Q0 +P1 | -01 +10 | +U0 -V1
+Q0 +Q1 | +10 | +V0 +V1
+P1 | +11 -01 | +S1
+R1 | -11 +10 | +V1
"""

IN_ROWS = 96
IN_ARRIVAL = (2, 4, 6)
MIX_ROWS = 144
SCORE_DELAY = 240
VALUE_DELAY = 260
SOFTMAX_DELAY = 780


def _parse_scheme(text):
    sign = {"+": 1, "-": -1}
    products, slots = [], 0
    for line in text.strip().split("\n"):
        left, weight, out = (part.split() for part in line.split("|"))
        left = [(sign[t[0]], t[1], int(t[2])) for t in left]
        weight = [(sign[t[0]], int(t[1]), int(t[2])) for t in weight]
        out = [(sign[t[0]], t[1], int(t[2])) for t in out]
        if len(weight) == 1:
            out = [(s * weight[0][0], b, n) for s, b, n in out]
            products.append((left, [(1,) + weight[0][1:]], out, None))
        else:
            products.append((left, sorted(weight, reverse=True), out, slots))
            slots += 1
    return products


def _signed_sum(terms):
    terms = sorted(terms, key=lambda t: -t[0])
    total = terms[0][1] if terms[0][0] > 0 else -terms[0][1]
    for s, v in terms[1:]:
        total = total + v if s > 0 else total - v
    return total


def _left_terms(left):
    return [(s * t, half, k) for s, b, k in left
            for t, half in {"P": [(1, 0)], "Q": [(1, 1)], "R": [(1, 0), (-1, 1)]}[b]]


def _scatter(acc, out, m):
    for s, b, n in out:
        if (b, n) not in acc:
            acc[b, n] = m if s > 0 else -m
        else:
            acc[b, n] = acc[b, n] + m if s > 0 else acc[b, n] - m


def _fast_matmul(scheme, product, direct, emit):
    acc = {}
    blocks = max(o[2] for p in scheme for o in p[2]) + 1
    last = {(half, n): max(r for r, p in enumerate(scheme) if any(o[1:] in (("UV"[half], n), ("S", n)) for o in p[2]))
            for half in range(2) for n in range(blocks)}
    for r, (_, _, out, _) in enumerate(scheme):
        _scatter(acc, out, product(r))
        for (half, n), when in last.items():
            if when == r:
                total = acc["UV"[half], n] + acc["S", n]
                emit(half, n, total if direct is None else total + direct(half, n))


def _dot(a, b):
    return jnp.dot(a, b, preferred_element_type=F32)


def _dot_nt(a, b):
    return lax.dot_general(a, b, (((1,), (1,)), ((), ())), preferred_element_type=F32)


def _stack(parts):
    return jnp.concatenate(parts, axis=0)


def _rows(i, n):
    if isinstance(i, int):
        return pl.ds(i * n, n)
    return pl.ds(pl.multiple_of(i * n, n), n)


def _matrix(words):
    return pltpu.bitcast(words, BF16)


def _put(ref, at, row, value, after=lambda v: v):
    if value.dtype == U32:
        ref[at + (pl.ds(row, value.shape[0]),)] = after(value)
        return
    for r in range(0, value.shape[0], 8):
        piece = after(value[r:r + 8]) if r % 16 else value[r:r + 8]
        ref[at + (pl.ds(row + r // 2, 4),)] = pltpu.bitcast(piece.astype(BF16), U32)


def _word_sum(terms):
    if len(terms) == 1 and terms[0][0] > 0:
        return terms[0][1]
    return _stack([_signed_sum([(s, _matrix(w)[r:r + 8].astype(F32)) for s, w in terms]) for r in (0, 8)])


def _spread(jobs, n):
    slots = [[] for _ in range(n)]
    total, spent = max(1, sum(cost for cost, _ in jobs)), 0
    for cost, job in jobs:
        slots[spent * n // total].append(job)
        spent += cost
    return slots


def _untimed(v):
    return v


_untimed.mark = lambda ref: None


def _at_once(jobs):
    for _, job in jobs:
        job(_untimed)


class _Stream:
    def __init__(self):
        self.now = 0
        self.waiting = []

    def defer(self, ready, cost, fn):
        self.waiting.append((ready, cost, fn))
        self.waiting.sort(key=lambda w: w[0])

    def _emit_next(self):
        ready, cost, fn = self.waiting.pop(0)
        self.now = max(self.now, ready) + cost
        fn()

    def run(self, cost, fn):
        while self.waiting and self.waiting[0][0] <= self.now:
            self._emit_next()
        self.now += cost
        return fn()

    def until(self, done):
        while not done():
            self._emit_next()


def _kernel(
    x_hbm, mem_hbm, wq_hbm, wk_hbm, wv_hbm, wo_hbm, wint_hbm, wsp_hbm, b_hbm, wout_hbm,
    out_hbm,
    x_v, lna_v, lnb_v, xn_w, xa_w, xb_w, mem_v, wint_w, win_w, wsp_w, wout_v, woutt_w, wol_w, b_v, bias_v,
    z1_v, d_v, z2_w, ws_w, ya_w, yb_w, gate_v, wqkv_w, wo_w, wfq_w, wfo_w,
    lq_w, lo_w, qkv_carry, o_carry, o16_w, o32_v, out_v, zero,
    sem_x, sem_in, sem_small, sem_sp, sem_qkv, sem_wo, sem_out,
    *, seg,
):
    S, D = out_v.shape
    M = mem_v.shape[0]
    H = o_carry.shape[0]
    DH = LANES
    FH = wout_v.shape[0]
    HF = FH // 2
    NTB = S // LANES
    NQ = NTB // 4
    NN = D // LANES
    assert (M, seg, NN, H, NQ) == (8, 32, 5, 32, 4)
    scheme5, scheme4, scheme2 = map(_parse_scheme, (_SCHEME_5, _SCHEME_4, _SCHEME_2))
    n2 = len(scheme2)
    n_five = H // NN

    def x_copy(i):
        r0, r1 = (2 * i, 2 * i + 2) if i < 2 else (4 * i - 4, 4 * i)
        rows = pl.ds(r0 * LANES, (r1 - r0) * LANES)
        return pltpu.make_async_copy(x_hbm.at[rows], x_v.at[rows], sem_x.at[i])

    cuts = [0] + [c * IN_ROWS for c in IN_ARRIVAL] + [FH]

    def win_copies(c):
        rows = [pl.ds((half * FH + cuts[c]) // 2, (cuts[c + 1] - cuts[c]) // 2) for half in range(2)]
        return [pltpu.make_async_copy(wint_hbm.bitcast(U32).at[r], wint_w.at[r], sem_in.at[c]) for r in rows]

    def wsp_copy(i):
        rows = _rows(i, 2 * LANES)
        return pltpu.make_async_copy(wsp_hbm.bitcast(U32).at[rows], wsp_w.at[rows], sem_sp.at[i])

    chunks = [range(NN * i, min(NN * (i + 1), H // 2)) for i in range(NQ)]

    def wo_copy(i):
        rows = pl.ds(chunks[i][0] * DH, len(chunks[i]) * DH)
        return pltpu.make_async_copy(wo_hbm.bitcast(U32).at[rows], wo_w.at[rows], sem_wo.at[i])

    def start_attention_weights(i):
        wo_copy(i).start()
        for j in chunks[i]:
            for m, w in enumerate((wk_hbm, wq_hbm, wv_hbm)):
                for b in range(2):
                    pltpu.make_async_copy(
                        w.bitcast(U32).at[:, b, j, :], wqkv_w.at[6 * j + 3 * b + m], sem_qkv.at[i]).start()

    def wait_attention_weights(i):
        wo_copy(i).wait()
        filled = wqkv_w.at[pl.ds(6 * chunks[i][0], 6 * len(chunks[i]))]
        pltpu.make_async_copy(filled, filled, sem_qkv.at[i]).wait()

    small_copies = [pltpu.make_async_copy(src, dst, sem_small.at[0])
                    for src, dst in ((wout_hbm, wout_v), (b_hbm, b_v), (mem_hbm, mem_v))]

    for e in range(zero.shape[0]):
        zero[e] = 0
    x_copy(0).start()
    for c in range(len(cuts) - 1):
        for cp in win_copies(c):
            cp.start()
    x_copy(1).start()

    def timed_after(result):
        always = jnp.full((8, LANES), zero[zero.shape[0] - 1], jnp.int32) == 0

        def after(v):
            reps = (v.shape[0] // 8, v.shape[1] // LANES)
            token = pltpu.bitcast(result[:8, :LANES], v.dtype)
            return jnp.where(jnp.tile(always, reps), v, jnp.tile(token, reps))

        marked = []

        def mark(ref):
            if not any(ref is other for other in marked):
                marked.append(ref)
                at = (ref.shape[0] - 1 + zero[zero.shape[0] - 1],) + (0,) * (len(ref.shape) - 3) + (pl.ds(0, 8),)
                ref[at] = pltpu.bitcast(result[:8, :LANES], ref.dtype)

        after.mark = mark
        return after

    def run_jobs(groups, result):
        jobs = [job for group in groups for job in group]
        if jobs:
            after = timed_after(result)
            for job in jobs:
                job(after)

    KX = (NN - 1) // 2

    def norm_jobs(p, dst_w, ln_v):
        def rows(r, e):
            start = p * (2 * LANES) + pl.multiple_of(zero[e], 64) + r
            return x_v[pl.ds(start, 16), :].astype(F32)

        def mean(r, after):
            ln_v[0, pl.ds(r, 16), :] = after(jnp.broadcast_to(
                jnp.mean(rows(r, 0), axis=-1, keepdims=True), (16, LANES)))

        def centred(r, e):
            return rows(r, e) - jnp.tile(ln_v[0, pl.ds(r, 16), :], (1, NN))

        def scale(r, after):
            d = centred(r, 1)
            ln_v[1, pl.ds(r, 16), :] = after(jnp.broadcast_to(
                lax.rsqrt(jnp.mean(d * d, axis=-1, keepdims=True) + EPS), (16, LANES)))

        def apply(r, after):
            xn = centred(r, 2) * jnp.tile(ln_v[1, pl.ds(r, 16), :], (1, NN))
            for k in range(NN):
                _put(xn_w, (p * (2 * LANES // 16) + r // 16, k), 0, xn[:, k * LANES:(k + 1) * LANES], after)

        def operands(r, after):
            start = p * (2 * LANES // 16) + zero[3]
            w = {(n, k): xn_w[start + (n * LANES + r) // 16, k] for n in range(2) for k in range(NN)}
            after.mark(dst_w)
            for n in range(2):
                _put(dst_w, (n2 * KX + n,), r // 2, w[n, 2 * KX])
            for e, (_, weight, _, _) in enumerate(scheme2):
                for t in range(KX):
                    _put(dst_w, (e * KX + t,), r // 2, _word_sum([(s, w[n, k * KX + t]) for s, k, n in weight]))

        both = range(0, 2 * LANES, 16)
        return ([(2, functools.partial(mean, r)) for r in both] + [(3, functools.partial(scale, r)) for r in both]
                + [(4, functools.partial(apply, r)) for r in both]
                + [(6, functools.partial(operands, r)) for r in range(0, LANES, 16)])

    def fold(z):
        return jnp.sum(z.reshape(z.shape[0] // 8, 8, LANES), axis=0)

    def in_proj(p, src, early=(), late=(), steady=(), before=lambda c: None, hold=0):
        n_chunks = FH // IN_ROWS
        per = n2 * KX + 4
        slots = iter(zip(*[[[]] * a + _spread(jobs, n_chunks * per - a - b) + [[]] * b
                           for jobs, a, b in ((early, hold * per, 30), (late, 40, 0), (steady, 0, 0))]))
        shift, s1, s2 = {}, {}, {}
        for c in range(n_chunks):
            rows = pl.ds(c * IN_ROWS, IN_ROWS)
            before(c)

            def tile(lhs, rhs):
                part = _dot_nt(_matrix(win_w[lhs, _rows(c, IN_ROWS // 2), :]), _matrix(src[rhs]))
                run_jobs(next(slots), part)
                return part

            def product(r):
                return _signed_sum([(1, tile(r * KX + t, r * KX + t)) for t in range(KX)])

            def direct(half, n):
                return tile(n2 * KX + half, n2 * KX + n)

            def emit(half, n, z):
                c0 = math.sqrt(2.0 / math.pi)
                z = z * (1.0 + jnp.tanh(z * (c0 + (c0 * 0.044715) * (z * z))))
                if half == 0:
                    z1_v[2 * p + n, rows, :] = z
                    return
                if c == 0:
                    shift[n] = z[:8]
                d = z - jnp.tile(shift[n], (IN_ROWS // 8, 1))
                d_v[2 * p + n, rows, :] = d
                s1[n] = fold(d) if c == 0 else s1[n] + fold(d)
                s2[n] = fold(d * d) if c == 0 else s2[n] + fold(d * d)

            _fast_matmul(scheme2, product, direct, emit)
        stats = []
        for n in range(2):
            off = jnp.sum(s1[n] + (FH // 8) * shift[n], axis=0, keepdims=True) * (1.0 / FH) - shift[n]
            var = jnp.sum(s2[n] - off * (2.0 * s1[n] - (FH // 8) * off), axis=0, keepdims=True) * (1.0 / FH)
            stats.append((off, 0.25 * lax.rsqrt(jnp.maximum(var, 0.0) + 4.0 * EPS)))
        return stats

    def rescale_jobs(q, stats, timed_input=False):
        def job(r, after):
            off = [jnp.tile(after(stats[n][0]) if timed_input else stats[n][0], (2, 1)) for n in range(4)]
            base = {}
            for k in range(4):
                for half in range(2):
                    base["PQ"[half], k] = (d_v[4 * q + k, pl.ds(half * HF + r, 16), :] - off[k]) * stats[k][1]
                base["R", k] = base["P", k] - base["Q", k]
            if not timed_input:
                after.mark(z2_w)
            for e, (left, _, _, _) in enumerate(scheme4):
                w = _signed_sum([(s, base[b, k]) for s, b, k in left])
                _put(z2_w, (q, e), r // 2, w)
            return w

        return [(1, functools.partial(job, r)) for r in range(0, HF, 16)]

    def weights_arrived(c):
        for cp in win_copies(c):
            cp.wait()
        if c == len(cuts) - 3:
            for i in range(2, NQ + 1):
                x_copy(i).start()
            for cp in small_copies:
                cp.start()
        if c == len(cuts) - 2:
            wsp_copy(0).start()
            wsp_copy(1).start()
            start_attention_weights(0)
            start_attention_weights(1)
        for r in range(cuts[c], cuts[c + 1], 16):
            w = [wint_w[pl.ds((half * FH + r) // 2, 8), :] for half in range(2)]
            for e, (left, _, _, _) in enumerate(scheme2):
                for t in range(KX):
                    _put(win_w, (e * KX + t,), r // 2, _word_sum(
                        [(s, w[half][:, (k * KX + t) * LANES:(k * KX + t + 1) * LANES])
                         for s, half, k in _left_terms(left)]))
            for half in range(2):
                _put(win_w, (n2 * KX + half,), r // 2, w[half][:, 2 * KX * LANES:])

    KY = HF // LANES * LANES
    DC = LANES // 2
    d_chunks = [(d, 2 * LANES + d) for d in range(0, 2 * LANES, DC)] + [(4 * LANES, 4 * LANES + DC)]

    def out_weight_jobs():
        def transpose(col, d, after):
            cols = pl.ds(d, LANES)
            if col < 2 * KY:
                w = wout_v[pl.ds(col // KY * HF + col % KY, LANES), cols]
            else:
                w = _stack([wout_v[pl.ds(k * HF + KY, HF - KY), cols] for k in range(2)])
            w = _matrix(after(pltpu.bitcast(w, U32)))
            woutt_w[pl.ds(d // 2, LANES // 2), pl.ds(col, w.shape[0])] = pltpu.bitcast(w.T, U32)

        def operands(c, r, after):
            w = [woutt_w[pl.ds((d + r) // 2, 8), pl.ds(0, 2 * KY)] for d in d_chunks[c]]
            after.mark(wol_w)
            for e, (left, _, _, _) in enumerate(scheme2):
                for t in range(0, KY, LANES):
                    _put(wol_w, (e, t // LANES), (c * DC + r) // 2, _word_sum(
                        [(s, w[half][:, k * KY + t:k * KY + t + LANES]) for s, half, k in _left_terms(left)]))

        return ([(2, functools.partial(transpose, col, d)) for d in range(0, D, LANES) for col in range(0, FH, LANES)]
                + [(4, functools.partial(operands, c, r)) for c in range(len(d_chunks)) for r in range(0, DC, 16)])

    def stage_jobs(o):
        def job(r, q, after):
            w = {(k, n): wsp_w[pl.ds(o * (2 * LANES) + (n * LANES + r) // 2, 8), pl.ds((4 * q + k) * LANES, LANES)]
                 for k in range(4) for n in range(4)}
            for e, (_, weight, _, _) in enumerate(scheme4):
                _put(ws_w, (e, q), r // 2, _word_sum([(s, w[k, n]) for s, k, n in weight]), after)

        return [(1, functools.partial(job, r, q)) for q in range(NQ) for r in range(0, LANES, 16)]

    x_copy(0).wait()
    for r in range(0, 2 * LANES, 16):
        x = x_v[pl.ds(r, 16), :].astype(F32)
        d = x - jnp.mean(x, axis=-1, keepdims=True)
        xn = d * lax.rsqrt(jnp.mean(d * d, axis=-1, keepdims=True) + EPS)
        for k in range(NN):
            _put(xn_w, (r // 16, k), 0, xn[:, k * LANES:(k + 1) * LANES])
    _at_once(norm_jobs(0, xa_w, lna_v)[-LANES // 16:])

    def before(c):
        if c * IN_ROWS in cuts:
            weights_arrived(cuts.index(c * IN_ROWS))
        if c == IN_ARRIVAL[-1]:
            x_copy(1).wait()

    stats = in_proj(0, xa_w, early=norm_jobs(1, xb_w, lna_v), before=before, hold=IN_ARRIVAL[-1])

    def phase1(o, stats):
        for k in range(NQ - 1):
            @pl.when(o == k)
            def _():
                x_copy(k + 2).wait()

        ahead = norm_jobs(2 * o + 3, xb_w, lnb_v)
        odd = in_proj(2 * o + 1, xb_w, early=norm_jobs(2 * o + 2, xa_w, lna_v), steady=ahead[:32])
        return in_proj(2 * o + 2, xa_w, late=rescale_jobs(o, stats + odd), steady=ahead[32:])

    stats = lax.fori_loop(0, NQ - 1, phase1, stats)
    for cp in small_copies + [wsp_copy(0)]:
        cp.wait()
    for i in range(2, NQ):
        wsp_copy(i).start()
    start_attention_weights(2)
    stats = stats + in_proj(NTB // 2 - 1, xb_w, early=out_weight_jobs(), steady=stage_jobs(0))
    results = []
    for _, job in rescale_jobs(NQ - 1, stats, timed_input=True):
        results.append(job(timed_after(results[-2]) if len(results) >= 2 else _untimed))
    bias_v[...] = 0.25 * b_v[...].astype(F32)

    def repack_jobs(j):
        def job(m, r, after):
            t, rows = 6 * j + m, pl.ds(r, 8)
            after.mark(wqkv_w)
            a = wqkv_w[t, rows, :]
            b = wqkv_w[t + 3, rows, :]
            wqkv_w[t, rows, :] = (a & U32(0xFFFF)) | (b << 16)
            wqkv_w[t + 3, rows, :] = (a >> 16) | (b & U32(0xFFFF0000))

        return [(12, functools.partial(job, m, r)) for m in range(3) for r in range(0, D // 2, 8)]

    def weight_sum_jobs(load, ref, entry, part):
        def job(r, after):
            after.mark(ref)
            words = {}
            for _, weight, _, slot in scheme5:
                if slot is None:
                    continue
                for _, k, n in weight:
                    if (k, n) not in words:
                        words[k, n] = load(k, n, pl.multiple_of(part * (DH // 4) + r + zero[0], 8))
                _put(ref, (entry, slot, part), r, _word_sum([(s, words[k, n]) for s, k, n in weight]))

        return [(276, functools.partial(job, r)) for r in range(0, DH // 4, 8)]

    def qkv_sum_jobs(g, m, part):
        def load(k, n, r):
            return wqkv_w[3 * (NN * g + n) + m, pl.ds(r + k * (DH // 2), 8), :]

        return weight_sum_jobs(load, wfq_w, 3 * g + m, part)

    def out_sum_jobs(g, part):
        def load(k, n, r):
            return wo_w[pl.ds(g * (NN * DH // 2) + r + k * (DH // 2), 8), pl.ds(n * LANES, LANES)]

        return weight_sum_jobs(load, wfo_w, g, part)

    def mix(o, jobs):
        rc = MIX_ROWS
        slots = iter(_spread(jobs, HF // rc * len(scheme4) * NQ))
        for c in range(HF // rc):
            ys = {}

            def product(r):
                total = None
                for q in range(NQ):
                    part = _dot_nt(_matrix(z2_w[q, r, _rows(c, rc // 2), :]), _matrix(ws_w[r, q]))
                    total = part if q == 0 else total + part
                    run_jobs([next(slots)], part)
                return total

            def emit(half, n, g):
                ys[half, n] = z1_v[4 * o + n, pl.ds(half * HF + c * rc, rc), :] * (g + bias_v[pl.ds(4 * o + n, 1), :])
                u = n // 2
                if not all((k, 2 * u + t) in ys for k in range(2) for t in range(2)):
                    return
                y_w = (ya_w, yb_w)[u]
                m = max(0, min(rc, KY - c * rc))
                if m:
                    for e, (_, weight, _, _) in enumerate(scheme2):
                        _put(y_w, (e,), c * rc // 2, _signed_sum([(s, ys[k, 2 * u + t][:m]) for s, k, t in weight]))
                if m < rc:
                    for k in range(2):
                        for t in range(2):
                            _put(y_w, (n2 + t,), (k * (HF - KY) + c * rc + m - KY) // 2, ys[k, 2 * u + t][m:])

            _fast_matmul(scheme4, product, None, emit)

    def out_proj(p, y_w, jobs):
        slots = iter(_spread(jobs, len(d_chunks) * n2))
        tiles = {}
        for c, d0 in enumerate(d_chunks):
            def part(r, k0, k1):
                lhs = [_matrix(wol_w[r, k // LANES, _rows(c, DC // 2), :]) for k in range(k0, k1, LANES)]
                total = _dot(jnp.concatenate(lhs, axis=1), _matrix(y_w[r, pl.ds(k0 // 2, (k1 - k0) // 2), :]))
                if k1 == KY:
                    run_jobs([next(slots)], total)
                return total

            early = [part(r, 0, KY - LANES) for r in range(3)] if c == 0 else []

            def product(r):
                return early[r] + part(r, KY - LANES, KY) if r < len(early) else part(r, 0, KY)

            def direct(half, n):
                return _dot(_matrix(woutt_w[pl.ds(d0[half] // 2, DC // 2), pl.ds(2 * KY, FH - 2 * KY)]),
                            _matrix(y_w[n2 + n, pl.ds(0, HF - KY), :]))

            def emit(half, n, h):
                d = d0[half] // LANES * LANES
                done = tiles.setdefault((d, n), {})
                done[d0[half]] = h + h * jnp.tanh(h)
                if len(done) * DC == LANES:
                    gate_v[_rows(2 * p + n, LANES), pl.ds(d, LANES)] = _stack([done[k] for k in sorted(done)]).T

            _fast_matmul(scheme2, product, direct, emit)

    def phase2(o, _):
        for k in range(NQ):
            @pl.when(o == k)
            def _():
                if k + 1 < NQ:
                    wsp_copy(k + 1).wait()
                wait_attention_weights(k)
                if k == 1:
                    start_attention_weights(3)

        whole, shared = (3 * o + 1) // 2, o // 2 * 3 + 1
        first = out_sum_jobs(whole, 0) + out_sum_jobs(whole, 1)
        repack = [job for u in range(NN) for job in repack_jobs(jnp.minimum(o * NN + u, H // 2) if u else o * NN)]
        jobs = [job for a, b in zip(first, _spread([(1, job) for job in repack], len(first))) for job in [a] + b]
        for m in range(3):
            jobs += qkv_sum_jobs(whole, m, 0) + qkv_sum_jobs(whole, m, 1) + qkv_sum_jobs(shared, m, o % 2)
        jobs += out_sum_jobs(shared, o % 2)
        mix(o, jobs)
        ahead = _spread([(1, job) for job in stage_jobs(jnp.minimum(o + 1, NQ - 1))], 2)
        out_proj(2 * o, ya_w, ahead[0])
        out_proj(2 * o + 1, yb_w, ahead[1])

    lax.fori_loop(0, NQ, phase2, None)

    L = M + seg
    T = seg - M
    row = lax.broadcasted_iota(jnp.int32, (L, L), 0)
    col = lax.broadcasted_iota(jnp.int32, (L, L), 1)
    keep = (row < M) | (row >= col)
    heads = list(range(NN * n_five, H)) + list(range(NN * n_five))
    order = [3 * (hd + b) + m for hd in heads[::2] for m in range(3) for b in range(2)]
    last_use = [max(r for r, p in enumerate(scheme5) if any(o[2] == n for o in p[2])) for n in range(NN)]

    def left_sum_jobs(block, store):
        base = {}

        def term(b, k):
            if (b, k) not in base:
                base[b, k] = term("P", k) - term("Q", k) if b == "R" else block("PQ".index(b), k)
            return base[b, k]

        def job(r, left, after):
            total = _signed_sum([(s, term(b, k)) for s, b, k in left])
            store(r, after(pltpu.bitcast(total.astype(BF16), U32)))

        return [(1, functools.partial(job, r, left)) for r, (left, _, _, _) in enumerate(scheme5)]

    def gather(acc, n):
        return _stack([acc["U", n] + acc["S", n], acc["V", n] + acc["S", n]])

    def four_segments(grp, mem):
        t0 = pl.multiple_of(grp * 4 * seg, 4 * seg)
        mxu = _Stream()

        def tokens(r, n, k):
            return _stack([_matrix(xn_w[grp * (4 * seg // 16) + e // 16, k]) for e in range(r, r + n, 16)]).astype(F32)

        def finish(r, n, k, s):
            rows, cols = pl.ds(t0 + r, n), pl.ds(k * LANES, LANES)
            out_v[rows, cols] = (x_v[rows, cols].astype(F32) + s * gate_v[rows, cols]).astype(out_v.dtype)

        for j in range(4):
            tiles = {}
            done = {}

            def attend(hd, j=j, tiles=tiles, done=done):
                st = {}

                def scores():
                    sc = _dot_nt(tiles.pop(3 * hd + 1), tiles.pop(3 * hd).astype(BF16))
                    sc = jnp.where(keep, sc * (DH ** -0.5 * LOG2E), -1e9 * LOG2E)
                    p = jnp.exp2(sc - jnp.max(sc, axis=1, keepdims=True))
                    st["p"] = p * pl.reciprocal(jnp.sum(p, axis=1, keepdims=True), approx=False, full_range=False)
                    st["t"] = mxu.now + SOFTMAX_DELAY
                    values_ready()

                def values_ready():
                    if "p" in st and 3 * hd + 2 in tiles:
                        mxu.defer(max(st["t"], done["v", hd] + VALUE_DELAY), L // 4, values)

                def values():
                    o = _dot(st.pop("p"), tiles.pop(3 * hd + 2).astype(BF16))
                    parts = [o[:M]] + ([o_carry[hd, pl.ds(0, M * j), :]] if j else [])
                    if j < 3:
                        new = T - M * j
                        o16_w[:, pl.ds(hd * DH, DH)] = pltpu.bitcast(_stack(parts + [o[M:M + new]]).astype(BF16), U32)
                        o_carry[hd, pl.ds(0, seg - new), :] = o[M + new:]
                    else:
                        o32_v[hd] = _stack(parts + [o[M:]])
                    done["o", hd] = mxu.now
                    g = hd // NN
                    if j == 3 and g < n_five and all(("o", NN * g + k) in done for k in range(NN)):
                        def keep_left(r, a):
                            lo_w[r, :, pl.ds(g * DH, DH)] = a

                        _at_once(left_sum_jobs(lambda t, k: o32_v[NN * g + k, pl.ds(t * seg, seg), :], keep_left))

                def on_tile(m):
                    if m == 1:
                        mxu.defer(mxu.now + SCORE_DELAY, L // 4, scores)
                    elif m == 2:
                        done["v", hd] = mxu.now
                        values_ready()

                return on_tile

            notify = [attend(hd) for hd in range(H)]

            def tile_done(t, y, j=j, tiles=tiles, notify=notify):
                old = 0 if j == 0 else T - M * (j - 1)
                parts = [y[:M]] + ([qkv_carry[t, pl.ds(0, old), :]] if old else [])
                tiles[t] = _stack(parts + [y[M:M + seg - old]])
                if j < 3:
                    qkv_carry[t, pl.ds(0, T - M * j), :] = y[M + seg - old:]
                notify[t // 3](t % 3)

            def need(hds, done=done):
                mxu.until(lambda: all(("o", hd) in done for hd in hds))

            if j == 0:
                h = [_stack([mem[k], tokens(0, 2 * seg, k)[:seg + T]]) for k in range(NN)]
                hh = jnp.concatenate(h, axis=1).astype(BF16)

                def keep_left(r, a):
                    lq_w[r] = a

                plain = order[:3 * (H - NN * n_five)]
                slots = iter(_spread(left_sum_jobs(lambda t, k: h[k][t * seg:(t + 1) * seg], keep_left),
                                     len(plain) * NN - 2) + [[]] * 2)
                for t in plain:
                    for k in range(NN):
                        part = mxu.run(seg // 2, lambda: _dot(
                            hh[:, k * LANES:(k + 1) * LANES],
                            _matrix(wqkv_w[t, _rows(k, DH // 2), :])))
                        y = part if k == 0 else y + part
                        run_jobs([next(slots)], part)
                    tile_done(t, y)
                for g in range(n_five):
                    for m in range(3):
                        first = 3 * NN * g + m
                        acc = {}
                        for r, (_, weight, out, slot) in enumerate(scheme5):
                            def product():
                                if slot is None:
                                    _, k, n = weight[0]
                                    w = wqkv_w[first + 3 * n, _rows(k, DH // 2), :]
                                else:
                                    w = _stack([wfq_w[3 * g + m, slot, e] for e in range(2)])
                                return _dot(_matrix(lq_w[r]), _matrix(w))

                            _scatter(acc, out, mxu.run(seg // 4, product))
                            for n in range(NN):
                                if last_use[n] == r:
                                    tile_done(first + 3 * n, gather(acc, n))
            else:
                r0 = seg + T * j
                a0 = r0 // 16 * 16
                h = [_stack([mem[k], tokens(a0, seg, k)[r0 - a0:r0 - a0 + T]]).astype(BF16) for k in range(NN)]
                partial = {}
                for k in range(NN):
                    for t in order[:4]:
                        y = mxu.run(seg // 4, lambda: _dot(
                            h[k], _matrix(wqkv_w[t, _rows(k, DH // 2), :])))
                        partial[t] = y if k == 0 else partial[t] + y
                        if k == NN - 1:
                            tile_done(t, partial.pop(t))
                hh = jnp.concatenate(h, axis=1)
                for t in order[4:]:
                    tile_done(t, mxu.run(NN * seg // 4, lambda: _dot(hh, _matrix(wqkv_w[t]))))

            if j < 3:
                total = [None] * NN

                def project(hd, n):
                    need([hd])
                    y = mxu.run(seg // 4, lambda: _dot(
                        _matrix(o16_w[:, pl.ds(hd * DH, DH)]),
                        _matrix(wo_w[_rows(hd, DH // 2), pl.ds(n * LANES, LANES)])))
                    total[n] = y if total[n] is None else total[n] + y

                for hd in heads[:-8]:
                    for n in range(NN):
                        project(hd, n)
                for n in range(NN):
                    for hd in heads[-8:]:
                        project(hd, n)
                    finish(T * j, T, n, total[n][M:])
                mem = [a[:M] for a in total]
            else:
                acc = {}
                mem = [None] * NN
                rest = range(NN * n_five, H)
                need(rest)
                o_rest = jnp.concatenate([o32_v[hd] for hd in rest], axis=1).astype(BF16)
                for n in range(NN):
                    y = mxu.run(len(rest) * seg // 2, lambda: _dot(
                        o_rest, _matrix(wo_w[pl.ds(rest[0] * DH // 2, len(rest) * DH // 2), pl.ds(n * LANES, LANES)])))
                    _scatter(acc, [(1, "U", n)], y[:seg])
                    _scatter(acc, [(1, "V", n)], y[seg:])
                for g0, g1 in ((0, n_five // 2), (n_five // 2, n_five)):
                    need(range(NN * g0, NN * g1))
                    span = pl.ds(g0 * DH, (g1 - g0) * DH)
                    for r, (_, weight, out, slot) in enumerate(scheme5):
                        def product():
                            if slot is None:
                                _, k, n = weight[0]
                                w = [wo_w[_rows(NN * g + k, DH // 2), pl.ds(n * LANES, LANES)] for g in range(g0, g1)]
                            else:
                                w = [wfo_w[g, slot, e] for g in range(g0, g1) for e in range(2)]
                            return _dot(_matrix(lo_w[r, :, span]), _matrix(_stack(w)))

                        _scatter(acc, out, mxu.run((g1 - g0) * seg // 4, product))
                        for n in range(NN):
                            if g1 == n_five and last_use[n] == r:
                                y = gather(acc, n)
                                finish(3 * T, seg + T, n, y[M:])
                                mem[n] = y[:M]
            assert not tiles and not mxu.waiting
            if j >= 2:
                rows = pl.ds(t0 + (j - 2) * 2 * seg, 2 * seg)
                pltpu.make_async_copy(out_v.at[rows], out_hbm.at[rows], sem_out.at[0]).start()
        return mem

    mem0 = mem_v[...].astype(F32)
    lax.fori_loop(0, S // (4 * seg), four_segments, [mem0[:, n * LANES:(n + 1) * LANES] for n in range(NN)])
    pltpu.make_async_copy(out_v, out_hbm, sem_out.at[0]).wait()


@functools.partial(jax.jit, static_argnames=("A_seg_len",))
def pallas_recurrent_scan__memory_aug_recurrent_mem_tr__mixer_gmlp__prompt_kernel(
    A_x, A_mem0, A_Wq, A_Wk, A_Wv, A_Wo, A_seg_len, B_x, B_w_in, B_w_sp, B_b_sp, B_w_out,
):
    del B_x
    B, S, D = A_x.shape
    M = A_mem0.shape[1]
    H, DH = A_Wq.shape[1], A_Wq.shape[2]
    FH = B_w_out.shape[0]
    seg = int(A_seg_len)
    assert B == 1 and DH == LANES
    ntb = S // LANES
    n5, n4, n2 = (len(_parse_scheme(text)) for text in (_SCHEME_5, _SCHEME_4, _SCHEME_2))
    n_sums = sum(p[3] is not None for p in _parse_scheme(_SCHEME_5))
    n_five = H // (D // LANES)
    x_tiles = n2 * ((D // LANES - 1) // 2) + 2
    ky = FH // 2 // LANES * LANES
    vmem, dma = pltpu.VMEM, pltpu.SemaphoreType.DMA
    scratch = [
        vmem((S, D), BF16),
        *[vmem((3, 2 * LANES, LANES), F32)] * 2,
        vmem((S // 16 + 1, D // LANES, 8, LANES), U32),
        *[vmem((x_tiles + 1, LANES // 2, LANES), U32)] * 2,
        vmem((M, D), BF16),
        vmem((FH, D), U32),
        vmem((x_tiles, FH // 2, LANES), U32),
        vmem((S // 2, S), U32),
        vmem((FH, D), BF16),
        vmem((D // 2, FH), U32),
        vmem((n2 + 1, ky // LANES, D // 4, LANES), U32),
        vmem((ntb, LANES), BF16),
        vmem((ntb, LANES), F32),
        *[vmem((ntb, FH, LANES), F32)] * 2,
        vmem((ntb // 4 + 1, n4, FH // 4, LANES), U32),
        vmem((n4 + 1, ntb // 4, LANES // 2, LANES), U32),
        *[vmem((n2 + 2, ky // 2, LANES), U32)] * 2,
        vmem((S + 16, D), F32),
        vmem((3 * H + 6, D // 2, DH), U32),
        vmem((H * DH // 2 + 16, D), U32),
        vmem((3 * n_five + 1, n_sums, 2, DH // 4, LANES), U32),
        vmem((n_five + 1, n_sums, 2, DH // 4, LANES), U32),
        vmem((n5 + 1, seg // 2, LANES), U32),
        vmem((n5, seg // 2, n_five * DH), U32),
        vmem((3 * H, seg - M, DH), F32),
        vmem((H, seg - M, DH), F32),
        vmem((seg // 2, H * DH), U32),
        vmem((H, 2 * seg, DH), F32),
        vmem((S, D), A_x.dtype),
        pltpu.SMEM((8,), jnp.int32),
        dma((ntb // 4 + 1,)), dma((len(IN_ARRIVAL) + 1,)), dma((1,)),
        dma((ntb // 4,)), dma((ntb // 4,)), dma((ntb // 4,)), dma((1,)),
    ]
    hbm = pl.BlockSpec(memory_space=pltpu.HBM)
    out = pl.pallas_call(
        functools.partial(_kernel, seg=seg),
        out_shape=jax.ShapeDtypeStruct((S, D), A_x.dtype),
        in_specs=[hbm] * 10,
        out_specs=hbm,
        scratch_shapes=scratch,
        compiler_params=pltpu.CompilerParams(vmem_limit_bytes=127 * 2**20),
    )(
        A_x.reshape(S, D),
        A_mem0.reshape(M, D),
        A_Wq.reshape(D // 2, 2, H, DH),
        A_Wk.reshape(D // 2, 2, H, DH),
        A_Wv.reshape(D // 2, 2, H, DH),
        A_Wo.reshape(H * DH, D),
        B_w_in.T,
        B_w_sp,
        B_b_sp.reshape(ntb, LANES),
        B_w_out,
    )
    return out.reshape(B, S, D)
```
